```python
import jax
import jax.numpy as jnp

def _softmax(x, axis=-1):
    return jax.nn.softmax(x, axis=axis)
def _gelu(x):
    return jax.nn.gelu(x, approximate=True)
def _silu(x):
    return jax.nn.silu(x)
def _sigmoid(x):
    return jax.nn.sigmoid(x)
def _layernorm(x, axis=-1, eps=1e-5):
    m = jnp.mean(x, axis=axis, keepdims=True)
    v = jnp.var(x, axis=axis, keepdims=True)
    return (x - m) / jnp.sqrt(v + eps)
def _scatter_add(tgt, idx, src, axis=0):
    return tgt.at[idx].add(src)
def _segment_sum(src, seg, n):
    return jax.ops.segment_sum(src, seg, n)
class _Rng:
    def __init__(self, key):
        self._k = key
    def _next(self):
        self._k, sub = jax.random.split(self._k)
        return sub
    def normal(self, shape):
        return jax.random.normal(self._next(), shape, dtype=jnp.bfloat16)
    def randint(self, lo, hi, shape):
        return jax.random.randint(self._next(), shape, lo, hi, dtype=jnp.int32)
    def uniform(self, shape, lo=0.0, hi=1.0):
        return jax.random.uniform(self._next(), shape, jnp.bfloat16, lo, hi)
    def permutation(self, n):
        return jax.random.permutation(self._next(), n)


kernel_name = 'interleave_layers__sliding_block__moe_arch_mod__prompt'

def setup_inputs():
    _rng = _Rng(jax.random.key(int.from_bytes(__import__("os").urandom(4), "little")))
    _w = (lambda a: (lambda t: t.astype(jnp.bfloat16) if jnp.issubdtype(t.dtype, jnp.floating) else t)(jnp.asarray(a)))
    def _A_setup():
        B, S, D = 1, 2048, 1024
        return {
            "x": _w((lambda *s: _rng.normal(s) * 0.05)(B, S, D)),
            "wqkv": _w((lambda *s: _rng.normal(s) * 0.05)(D, 3 * D)),
            "wo": _w((lambda *s: _rng.normal(s) * 0.05)(D, D)),
        }
    _A_in = _A_setup()

    def _B_setup():
        B, S, D, F, C = 1, 2048, 1024, 3584, 1
        return {
            "x": _w((lambda *s: _rng.normal(s) * 0.05)(B, S, D)),
            "w_r": _w((lambda *s: _rng.normal(s) * 0.05)(D)),
            "w_gate": _w((lambda *s: _rng.normal(s) * 0.05)(D, F)),
            "w_up": _w((lambda *s: _rng.normal(s) * 0.05)(D, F)),
            "w_down": _w((lambda *s: _rng.normal(s) * 0.05)(F, D)),
        }
    _B_in = _B_setup()

    return {
        "A_x": _A_in["x"],
        "A_wqkv": _A_in["wqkv"],
        "A_wo": _A_in["wo"],
        "B_x": _B_in["x"],
        "B_w_r": _B_in["w_r"],
        "B_w_gate": _B_in["w_gate"],
        "B_w_up": _B_in["w_up"],
        "B_w_down": _B_in["w_down"],
    }

def reference(A_x, A_wqkv, A_wo, B_x, B_w_r, B_w_gate, B_w_up, B_w_down):
    def _A_ref(x, wqkv, wo):
        B, S, D = x.shape
        H = 32; Dh = D // H; W = 256
        qkv = (lambda x, *d: x.transpose(*d))((x @ wqkv).reshape(B, S, 3, H, Dh), 2, 0, 3, 1, 4)
        q, k, v = qkv[0], qkv[1], qkv[2]
        scores = jnp.einsum("bhqd,bhkd->bhqk", q, k) * (Dh ** -0.5)
        idx = jnp.arange(S)
        mask = (idx[:, None] - idx[None, :] >= 0) & (idx[:, None] - idx[None, :] < W)
        scores = jnp.where(mask[None, None], scores, -1e9)
        p = _softmax(scores, axis=-1)
        o = jnp.einsum("bhqk,bhkd->bhqd", p, v)
        return (lambda x, *d: x.transpose(*d))(o, 0, 2, 1, 3).reshape(B, S, D) @ wo

    def _B_ref(x, w_r, w_gate, w_up, w_down):
        B, S, D = x.shape
        C = 1
        r = x @ w_r
        idx = jnp.argsort(-r, axis=-1)[:, :C]
        idx_e = jnp.repeat(idx.reshape(B, C, 1), D, axis=2)
        x_sel = jnp.take_along_axis(x, idx_e, axis=1)
        g = _silu(x_sel @ w_gate)
        u = x_sel @ w_up
        y = (g * u) @ w_down
        r_sel = _sigmoid(jnp.take_along_axis(r, idx, axis=1))
        y = y * r_sel.reshape(B, C, 1)
        b_off = (jnp.arange(B) * S).reshape(B, 1)
        flat_idx = (idx + b_off).reshape(B * C)
        zero = (x * 0.0).reshape(B * S, D)
        upd = _scatter_add(zero, flat_idx, y.reshape(B * C, D), axis=0)
        return x + upd.reshape(B, S, D)

    x = A_x
    x = x + _A_ref(_layernorm(x, axis=-1), A_wqkv, A_wo)
    x = x + _B_ref(_layernorm(x, axis=-1), B_w_r, B_w_gate, B_w_up, B_w_down)
    x = x + _A_ref(_layernorm(x, axis=-1), A_wqkv, A_wo)
    x = x + _B_ref(_layernorm(x, axis=-1), B_w_r, B_w_gate, B_w_up, B_w_down)
    return x
```

```python
import functools
import numpy as np
import jax
import jax.numpy as jnp
from jax import lax
import jax.experimental.pallas as pl
import jax.experimental.pallas.tpu as pltpu

S, D, F = 2048, 1024, 3584
H, DH, W = 32, 32, 256
G = 8
EPS = 1e-5
QSCALE = float(DH ** -0.5 * np.log2(np.e))
RB = 512
BF = jnp.bfloat16
F32 = jnp.float32
NT = (((1,), (1,)), ((), ()))


def _ln(x):
    m = jnp.mean(x, axis=-1, keepdims=True)
    xc = x - m
    v = jnp.mean(xc * xc, axis=-1, keepdims=True)
    return xc * lax.rsqrt(v + EPS)


def kernel(x_hbm, wqkv_hbm, wo_hbm, wr_ref, wg_hbm, wu_hbm, wd_hbm, out_hbm,
           xin, xs, xn, xb, wqkv, wvt, wo, wg, wu, wd, q_s, k_s, vt_s, o_s, sems, osems):
    NB = S // RB
    cp_x = [pltpu.make_async_copy(x_hbm.at[pl.ds(i * RB, RB)], xin.at[pl.ds(i * RB, RB)], sems.at[i]) for i in range(NB)]
    cp_wqkv = pltpu.make_async_copy(wqkv_hbm, wqkv, sems.at[NB])
    cp_wo = pltpu.make_async_copy(wo_hbm, wo, sems.at[NB + 1])
    cp_wg = pltpu.make_async_copy(wg_hbm, wg, sems.at[NB + 2])
    cp_wu = pltpu.make_async_copy(wu_hbm, wu, sems.at[NB + 3])
    cp_wd = pltpu.make_async_copy(wd_hbm, wd, sems.at[NB + 4])
    cp_x[0].start()
    cp_wqkv.start()
    for c in cp_x[1:]:
        c.start()
    cp_wo.start()
    cp_wg.start()
    cp_wu.start()
    cp_wd.start()

    k_s[:, 0:W, :] = jnp.zeros((G, W, 128), BF)
    vt_s[:, 0:2] = jnp.zeros((G, 2, 128, 128), BF)

    for i in range(NB):
        cp_x[i].wait()

        def ln0(j, c, i=i):
            r0 = pl.multiple_of(i * RB + j * 64, 64)
            x = xin[pl.ds(r0, 64), :].astype(F32)
            xs[pl.ds(r0, 64), :] = x
            xn[pl.ds(r0, 64), :] = _ln(x).astype(BF)
            return c
        lax.fori_loop(0, RB // 64, ln0, 0)

    cp_wqkv.wait()

    def tr(j, c):
        c0 = pl.multiple_of(j * 128, 128)
        for kk in range(8):
            wvt[pl.ds(c0, 128), kk * 128:(kk + 1) * 128] = wqkv[kk * 128:(kk + 1) * 128, pl.ds(2 * D + c0, 128)].T
        return c
    lax.fori_loop(0, 8, tr, 0)

    lane = lax.broadcasted_iota(jnp.int32, (64, 128), 1)
    row = lax.broadcasted_iota(jnp.int32, (64, 128), 0)
    tri = row > (lane & 63)
    lo_half = lax.broadcasted_iota(jnp.int32, (64, 128), 1) < 64

    def qkv_block(i, c):
        r0 = pl.multiple_of(i * RB, RB)
        a = xn[pl.ds(r0, RB), :]
        q = jnp.dot(a, wqkv[:, 0:D], preferred_element_type=F32)
        q = (q * QSCALE).astype(BF)
        for g in range(G):
            q_s[g, pl.ds(r0, RB), :] = q[:, g * 128:(g + 1) * 128]
        k = jnp.dot(a, wqkv[:, D:2 * D], preferred_element_type=F32).astype(BF)
        for g in range(G):
            k_s[g, pl.ds(W + r0, RB), :] = k[:, g * 128:(g + 1) * 128]
        vt = lax.dot_general(wvt[...], a, NT, preferred_element_type=F32).astype(BF)
        for g in range(G):
            for j in range(RB // 128):
                vt_s[g, 2 + i * (RB // 128) + j] = vt[g * 128:(g + 1) * 128, j * 128:(j + 1) * 128]
        return c

    def softmax_t(s, nvalid_from):
        top = s[0:64]
        mid = s[64:256]
        if nvalid_from > 0:
            neg = jnp.full((64, 128), -1e30, F32)
            top = neg
            if nvalid_from > 64:
                mid = jnp.concatenate([neg] * ((nvalid_from - 64) // 64) + ([s[nvalid_from:256]] if nvalid_from < 256 else []), axis=0)
        e = jnp.where(tri, top, s[256:320])
        t = jnp.concatenate([e, mid], axis=0)
        m = jnp.max(t, axis=0, keepdims=True)
        p = jnp.exp2(t - m)
        l = jnp.sum(p, axis=0, keepdims=True)
        pb = p.astype(BF)
        zero = jnp.zeros((64, 128), BF)
        p0 = jnp.where(tri, pb[0:64], zero)
        p4 = jnp.where(tri, zero, pb[0:64])
        return [p0, pb[64:128], pb[128:192], pb[192:256], p4], l

    def attn_qblock(g, qb, first):
        q0 = qb * 128 if first else pl.multiple_of(qb * 128, 128)
        qq = q_s[g, pl.ds(q0, 128), :]
        kk = k_s[g, pl.ds(q0, 384), :]
        vt = jnp.concatenate([vt_s[g, qb + j] for j in range(3)], axis=1)
        hl = lax.broadcasted_iota(jnp.int32, (64, 128), 1) // DH
        zero = jnp.zeros((64, 128), BF)
        outs = []
        for hp in range(2):
            h0, h1 = 2 * hp, 2 * hp + 1
            qa, qb_ = qq[0:64], qq[64:128]
            wa = jnp.concatenate([jnp.where(hl == h0, qa, zero), jnp.where(hl == h1, qa, zero)], axis=0)
            wb = jnp.concatenate([jnp.where(hl == h1, qb_, zero), jnp.where(hl == h0, qb_, zero)], axis=0)
            sa = lax.dot_general(kk[0:320], wa, NT, preferred_element_type=F32)
            sb = lax.dot_general(kk[64:384], wb, NT, preferred_element_type=F32)
            va = max(0, 256 - qb * 128) if first else 0
            vb = max(0, 192 - qb * 128) if first else 0
            pa, la = softmax_t(sa, va)
            pb, lb = softmax_t(sb, vb)
            pa = pa + [zero]
            pb = [zero] + pb
            c = jnp.concatenate([jnp.where(lo_half, a_, b_) for a_, b_ in zip(pa, pb)], axis=0)
            d = jnp.concatenate([jnp.where(lo_half, b_, a_) for a_, b_ in zip(pa, pb)], axis=0)
            lo1 = lo_half[0:1]
            lc = jnp.where(lo1, la, lb)
            ld = jnp.where(lo1, lb, la)
            oc = jnp.dot(vt[h0 * DH:(h0 + 1) * DH], c, preferred_element_type=F32) * (1.0 / lc)
            od = jnp.dot(vt[h1 * DH:(h1 + 1) * DH], d, preferred_element_type=F32) * (1.0 / ld)
            outs += [oc, pltpu.roll(od, 64, axis=1)]
        ot = jnp.concatenate(outs, axis=0)
        o_s[pl.ds(q0, 128), pl.ds(pl.multiple_of(g * 128, 128), 128)] = ot.T.astype(BF)

    def attn_first(g, c):
        attn_qblock(g, 0, True)
        attn_qblock(g, 1, True)
        return c

    QPI = 2

    def attn_rest(it, c):
        g = it % G
        qb = 2 + (it // G) * QPI
        for j in range(QPI):
            attn_qblock(g, qb + j, False)
        return c

    wr = wr_ref[...].astype(F32)

    def layer(li, c):
        lax.fori_loop(0, NB, qkv_block, 0)
        lax.fori_loop(0, G, attn_first, 0)
        lax.fori_loop(0, G * (S // 128 - 2) // QPI, attn_rest, 0)

        @pl.when(li == 0)
        def _():
            cp_wo.wait()

        def out_block(i, carry):
            best, bidx = carry
            r0 = pl.multiple_of(i * RB, RB)
            x1 = xs[pl.ds(r0, RB), :] + jnp.dot(o_s[pl.ds(r0, RB), :], wo[...], preferred_element_type=F32)
            n1 = _ln(x1)
            n1b = n1.astype(BF)
            xb[pl.ds(r0, RB), :] = n1b
            r = jnp.sum(n1b.astype(F32) * wr, axis=-1, keepdims=True)
            x2 = x1 + n1
            xs[pl.ds(r0, RB), :] = x2
            xn[pl.ds(r0, RB), :] = _ln(x2).astype(BF)
            xin[pl.ds(r0, RB), :] = x2.astype(BF)
            rid = lax.broadcasted_iota(jnp.int32, (8, 1), 0) + r0
            for j in range(RB // 8):
                rj = r[j * 8:(j + 1) * 8]
                take = rj > best
                best = jnp.where(take, rj, best)
                bidx = jnp.where(take, rid + j * 8, bidx)

            @pl.when(li == 1)
            def _():
                pltpu.make_async_copy(xin.at[pl.ds(r0, RB)], out_hbm.at[pl.ds(r0, RB)], osems.at[i]).start()
            return best, bidx

        best, bidx = lax.fori_loop(0, NB, out_block,
                                   (jnp.full((8, 1), -jnp.inf, F32), jnp.zeros((8, 1), jnp.int32)))
        rmax = jnp.max(best, axis=0, keepdims=True)
        idx = jnp.min(jnp.where(best == rmax, bidx, S - 1))
        idx = jnp.clip(idx, 0, S - 1)

        @pl.when(li == 0)
        def _():
            cp_wg.wait()
            cp_wu.wait()
            cp_wd.wait()

        t0 = pl.multiple_of((idx // 16) * 16, 16)
        xsel = xb[pl.ds(t0, 16), :]
        gt = jnp.dot(xsel, wg[...], preferred_element_type=F32)
        ut = jnp.dot(xsel, wu[...], preferred_element_type=F32)
        hh = (gt * jax.nn.sigmoid(gt) * ut).astype(BF)
        y = jnp.dot(hh, wd[...], preferred_element_type=F32) * jax.nn.sigmoid(rmax)
        sel = lax.broadcasted_iota(jnp.int32, (16, D), 0) == (idx - t0)
        x3 = xs[pl.ds(t0, 16), :] + jnp.where(sel, y, 0.0)
        xs[pl.ds(t0, 16), :] = x3
        xn[pl.ds(t0, 16), :] = _ln(x3).astype(BF)

        @pl.when(li == 1)
        def _():
            for i in range(NB):
                pltpu.make_async_copy(xin.at[pl.ds(i * RB, RB)], out_hbm.at[pl.ds(i * RB, RB)], osems.at[i]).wait()
            xin[pl.ds(t0, 16), :] = x3.astype(BF)
            cp = pltpu.make_async_copy(xin.at[pl.ds(t0, 16)], out_hbm.at[pl.ds(t0, 16)], osems.at[0])
            cp.start()
            cp.wait()
        return c

    lax.fori_loop(0, 2, layer, 0)


@jax.jit
def pallas_interleave_layers__sliding_block__moe_arch_mod__prompt_kernel(
    A_x, A_wqkv, A_wo, B_x, B_w_r, B_w_gate, B_w_up, B_w_down):
    del B_x
    any_spec = pl.BlockSpec(memory_space=pl.ANY)
    out = pl.pallas_call(
        kernel,
        out_shape=jax.ShapeDtypeStruct((S, D), BF),
        in_specs=[any_spec, any_spec, any_spec, pl.BlockSpec(memory_space=pltpu.VMEM), any_spec, any_spec, any_spec],
        out_specs=any_spec,
        scratch_shapes=[
            pltpu.VMEM((S, D), BF),
            pltpu.VMEM((S, D), F32),
            pltpu.VMEM((S, D), BF),
            pltpu.VMEM((S, D), BF),
            pltpu.VMEM((D, 3 * D), BF),
            pltpu.VMEM((D, D), BF),
            pltpu.VMEM((D, D), BF),
            pltpu.VMEM((D, F), BF),
            pltpu.VMEM((D, F), BF),
            pltpu.VMEM((F, D), BF),
            pltpu.VMEM((G, S, 128), BF),
            pltpu.VMEM((G, S + W, 128), BF),
            pltpu.VMEM((G, S // 128 + 2, 128, 128), BF),
            pltpu.VMEM((S, D), BF),
            pltpu.SemaphoreType.DMA((S // RB + 5,)),
            pltpu.SemaphoreType.DMA((S // RB,)),
        ],
        compiler_params=pltpu.CompilerParams(vmem_limit_bytes=120 * 2**20),
        name="kern",
    )(A_x.reshape(S, D), A_wqkv, A_wo, B_w_r.reshape(1, D), B_w_gate, B_w_up, B_w_down)
    return out.reshape(1, S, D)
```

```python
import numpy as np
import jax
import jax.numpy as jnp
from jax import lax
import jax.experimental.pallas as pl
import jax.experimental.pallas.tpu as pltpu

S, D, F = 2048, 1024, 3584
DH, W = 32, 256
G = D // 128
FT = F // 128
R = 128
NB = S // R
EPS = 1e-5
QSCALE = float(DH ** -0.5 * np.log2(np.e))
NEG = -1e30
BF = jnp.bfloat16
F32 = jnp.float32
U32 = jnp.uint32
NT = (((1,), (1,)), ((), ()))
XC = 4


def _pk(x):
    return pltpu.bitcast(x.astype(BF), U32)


def _up(u):
    return pltpu.bitcast(u, BF)


def _rowsum(parts):
    s = parts[0]
    for p in parts[1:]:
        s = s + p
    return jnp.sum(s, axis=-1, keepdims=True)


def _center(parts):
    m = _rowsum(parts) * (1.0 / D)
    xc = [p - m for p in parts]
    v = _rowsum([c * c for c in xc]) * (1.0 / D)
    return xc, v


def kernel(x_hbm, wqkv_hbm, wo_hbm, wr_ref, wg_hbm, wu_hbm, wd_hbm, out_hbm,
           xio, xs, xn, wqkv, wvt, wo, wg, wu, wd, xn_new, o_s, wr_s, st_f, st_i, sems, osems, *grp):
    qkv_s, p_s = grp[:G], grp[G:]
    def col_copy(src, dst, j, sem):
        return pltpu.make_async_copy(src.at[:, pl.ds(j * 128, 128)], dst.at[j].bitcast(BF), sem)

    rc = S // XC
    xn_b, xnn_b, o_b, wvt_b = (r.bitcast(BF) for r in (xn, xn_new, o_s, wvt))
    qkv_b = [r.bitcast(BF) for r in qkv_s]
    p_b = [r.bitcast(BF) for r in p_s]

    def L(g):
        return slice(g * 128, (g + 1) * 128)
    cp_x = [[pltpu.make_async_copy(x_hbm.at[pl.ds(i * rc, rc), pl.ds(j * 128, 128)],
                                   xio.at[j, pl.ds(i * rc // 2, rc // 2)].bitcast(BF), sems.at[i])
             for j in range(G)] for i in range(XC)]
    cp_wqkv = [col_copy(wqkv_hbm, wqkv, j, sems.at[XC]) for j in range(3 * G)]
    cp_wo = [col_copy(wo_hbm, wo, j, sems.at[XC + 1]) for j in range(G)]
    cp_ffn = ([col_copy(wg_hbm, wg, j, sems.at[XC + 2]) for j in range(FT)]
              + [col_copy(wu_hbm, wu, j, sems.at[XC + 2]) for j in range(FT)]
              + [col_copy(wd_hbm, wd, j, sems.at[XC + 2]) for j in range(G)])
    for c in cp_x[0] + cp_wqkv + sum(cp_x[1:], []) + cp_wo + cp_ffn:
        c.start()

    for g in range(G):
        qkv_s[g][(S + W) // 2 + 32:(S + W) // 2 + 40, 0:128] = jnp.zeros((8, 128), U32)
        wr_s[g] = jnp.broadcast_to(wr_ref[g:g + 1, :].astype(F32), (16, 128))

    for i in range(XC):
        for c in cp_x[i]:
            c.wait()

        def ln0(j, c, i=i):
            r0 = pl.multiple_of(i * rc + j * 128, 128)
            h0 = pl.multiple_of(i * rc // 2 + j * 64, 64)
            x = [_up(xio[g, pl.ds(h0, 64), :]).astype(F32) for g in range(G)]
            xc, v = _center(x)
            rs = lax.rsqrt(v + EPS)
            for g in range(G):
                xs[g, pl.ds(r0, 128), :] = x[g]
                xn_b[pl.ds(r0, 128), L(g)] = (xc[g] * rs).astype(BF)
            return c
        lax.fori_loop(0, rc // 128, ln0, 0)

    for c in cp_wqkv:
        c.wait()

    def tr(j, c):
        for kk in range(G):
            wvt_b[pl.ds(pl.multiple_of(j * 128, 128), 128), L(kk)] = _up(wqkv[2 * G + j, kk * 64:(kk + 1) * 64, :]).T
        return c
    lax.fori_loop(0, G, tr, 0)
    for c in cp_wo:
        c.wait()

    lane64 = lax.broadcasted_iota(jnp.int32, (64, 128), 1)
    tri = lax.broadcasted_iota(jnp.int32, (64, 128), 0) > (lane64 & 63)
    lane32 = lax.broadcasted_iota(jnp.int32, (32, 128), 1)
    row32 = lax.broadcasted_iota(jnp.int32, (32, 128), 0)
    lo_half = lane32 < 64
    u0 = jnp.zeros((32, 128), U32)
    tri_p = (jnp.where(2 * row32 > (lane32 & 63), U32(0x0000FFFF), U32(0))
             | jnp.where(2 * row32 + 1 > (lane32 & 63), U32(0xFFFF0000), U32(0)))
    head_of_lane = lane32 // DH

    def lhs_tiles(ref, b):
        h0 = pl.multiple_of(b * (R // 2), R // 2)
        return _up(ref[pl.ds(h0, R // 2), :])

    ROWS = (S + W) // 2

    def put(b, g, col, off, val):
        for i in range(R // 16):
            qkv_b[g][pl.ds(pl.multiple_of(off + b * R + i * 16, 16), 16), L(col)] = val[i * 16:(i + 1) * 16].astype(BF)
            yield

    def q_piece(b, g):
        q = jnp.dot(lhs_tiles(xn, b), _up(wqkv[g]), preferred_element_type=F32)
        yield from put(b, g, 0, 0, q * QSCALE)

    def k_piece(b, g):
        k = jnp.dot(lhs_tiles(xn, b), _up(wqkv[G + g]), preferred_element_type=F32)
        yield from put(b, g, 1, W, k)

    def v_piece(b, g):
        vt = lax.dot_general(_up(wvt[g * 64:(g + 1) * 64, :]), lhs_tiles(xn, b), NT, preferred_element_type=F32)
        yield from put(b, g, 2, W, vt)

    def o_piece(b, g):
        y = jnp.dot(_up(o_s[...]), _up(wo[g]), preferred_element_type=F32)
        for i in range(R // 16):
            rows = pl.ds(pl.multiple_of(b * R + i * 16, 16), 16)
            xs[g, rows, :] = xs[g, rows, :] + y[i * 16:(i + 1) * 16]
            yield

    EP = 16

    def epi_piece(b, j):
        r0 = pl.multiple_of(b * R + j * EP, EP)
        h0 = pl.multiple_of(b * (R // 2) + j * (EP // 2), EP // 2)
        x1 = [xs[g, pl.ds(r0, EP), :] for g in range(G)]
        m = _rowsum(x1) * (1.0 / D)
        xc = [p - m for p in x1]
        v = _rowsum([c * c for c in xc]) * (1.0 / D)
        rs = lax.rsqrt(v + EPS)
        a = 1.0 + rs
        c2 = a * lax.rsqrt(v * a * a + EPS)
        r = rs * _rowsum([xc[g] * wr_s[g] for g in range(G)])
        for g in range(G):
            x2 = xc[g] * a + m
            xs[g, pl.ds(r0, EP), :] = x2
            xio[g, pl.ds(h0, EP // 2), :] = _pk(x2)
            xnn_b[j * EP:(j + 1) * EP, L(g)] = (xc[g] * c2).astype(BF)
        take = r > st_f[0]
        st_f[0] = jnp.where(take, r, st_f[0])
        st_f[1] = jnp.where(take, rs, st_f[1])
        st_i[...] = jnp.where(take, lax.broadcasted_iota(jnp.int32, (EP, 1), 0) + r0, st_i[...])

    def qk_piece(b, g):
        h0 = pl.multiple_of(b * 64, 64)
        qa = qkv_s[g][pl.ds(h0, 32), L(0)]
        qb = qkv_s[g][pl.ds(h0 + 32, 32), L(0)]
        res = []
        for hp in range(2):
            m0 = head_of_lane == 2 * hp
            m1 = head_of_lane == 2 * hp + 1
            wa = _up(jnp.concatenate([jnp.where(m0, qa, u0), jnp.where(m1, qa, u0)], axis=0))
            wb = _up(jnp.concatenate([jnp.where(m1, qb, u0), jnp.where(m0, qb, u0)], axis=0))
            for c, w in enumerate((wa, wb)):
                skip = max(0, 4 - 2 * b - c) if isinstance(b, int) else 0
                kk = _up(qkv_s[g][pl.ds(h0 + 32 * (c + skip), 32 * (5 - skip)), L(1)])
                sc = lax.dot_general(kk, w, NT, preferred_element_type=F32)
                e = jnp.where(tri, NEG if skip else sc[0:64], sc[-64:])
                mid = sc[(0 if skip else 64):-64]
                t = jnp.concatenate([e, mid], axis=0) if mid.shape[0] else e
                res.append((t, jnp.max(t, axis=0, keepdims=True)))
        return res

    def exp_work(g, sc, get_max, sums):
        for i, (t, _) in enumerate(sc):
            acc = None
            for u in range(t.shape[0] // 16):
                m = get_max(i)
                p = jnp.exp2(t[u * 16:(u + 1) * 16] - jnp.concatenate([m, m], axis=0))
                p_b[g][u * 16:(u + 1) * 16, L(i)] = p.astype(BF)
                p = p[0:8] + p[8:16]
                acc = p if acc is None else acc + p
                yield
            sums.append(jnp.sum(acc, axis=0, keepdims=True))

    def pv_piece(b, g, sc, sums):
        def chunks(i):
            n = sc[i][0].shape[0] // 64
            pe = p_s[g][0:32, L(i)]
            p0 = pe & tri_p
            return [p0] + [u0] * (4 - n) + [p_s[g][32 * j:32 * j + 32, L(i)] for j in range(1, n)] + [pe ^ p0]
        outs = []
        lo1 = lo_half[0:1]
        for hp in range(2):
            pa = chunks(2 * hp) + [u0]
            pb = [u0] + chunks(2 * hp + 1)
            la, lb = sums[2 * hp], sums[2 * hp + 1]
            for h, x_, y_, lx, ly in ((2 * hp, pa, pb, la, lb), (2 * hp + 1, pb, pa, lb, la)):
                j0 = max(0, 2 - b) if isinstance(b, int) else 0
                p = _up(jnp.concatenate([jnp.where(lo_half, x, y) for x, y in zip(x_[2 * j0:], y_[2 * j0:])], axis=0))
                vt = jnp.concatenate(
                    [_up(qkv_s[g][pl.ds(pl.multiple_of((b + j) * 64 + h * 16, 16), 16), L(2)]) for j in range(j0, 3)], axis=1)
                o = jnp.dot(vt, p, preferred_element_type=F32) * (1.0 / jnp.where(lo1, lx, ly))
                outs.append(o if h % 2 == 0 else pltpu.roll(o, 64, axis=1))
        o_b[:, L(g)] = jnp.concatenate(outs, axis=0).astype(BF).T

    def step(li, t, do_qkv, do_attn, do_out):
        def dense(g):
            if g == 0:
                return [o_piece(t - 1, i) for i in range(G)] if do_out else []
            return [f(t + 1, g - 1) for f in (q_piece, k_piece, v_piece)] if do_qkv else []

        if not (isinstance(t, int) and t < 2):
            xn[pl.ds(pl.multiple_of((t - 2) * (R // 2), R // 2), R // 2), :] = xn_new[...]
        if do_attn:
            sc = qk_piece(t, 0)
        for g in range(G + 1):
            pieces = dense(g)
            work, sums, nwork = iter(()), [], 0
            if do_attn and g < G:
                mx = [jnp.broadcast_to(m, (8, 128)) for _, m in sc]
                if not pieces:
                    get_max = lambda i, mx=mx: mx[i]
                elif g == 0:
                    for i in range(4):
                        xs[G - 1, S + 8 * i:S + 8 * i + 8, :] = mx[i]
                    get_max = lambda i: xs[G - 1, S + 8 * i:S + 8 * i + 8, :]
                else:
                    for i in range(4):
                        qkv_s[g - 1][ROWS + 8 * i:ROWS + 8 * i + 8, L(0)] = pltpu.bitcast(mx[i], U32)
                    get_max = lambda i, g=g: pltpu.bitcast(qkv_s[g - 1][ROWS + 8 * i:ROWS + 8 * i + 8, L(0)], F32)
                work = exp_work(g, sc, get_max, sums)
                nwork = sum(x.shape[0] // 16 for x, _ in sc)
            nch, done, ch = len(pieces) * (R // 16), 0, 0
            for pi, pc in enumerate(pieces):
                for _ in pc:
                    ch += 1
                    while done < nwork * ch // nch:
                        next(work)
                        done += 1
                if do_out and g >= 1 and pi == 0:
                    tok = pltpu.bitcast(qkv_s[g - 1][ROWS + 32:ROWS + 40, L(0)], F32)
                    xs[0, pl.ds(pl.multiple_of(S + 8 * li, 8), 8), :] = tok
                    epi_piece(t - 1, g - 1)
            if do_out and g >= 1 and not pieces:
                epi_piece(t - 1, g - 1)
            for _ in work:
                pass
            if do_attn and g < G:
                cur = sc
                if g + 1 < G:
                    sc = qk_piece(t, g + 1)
                pv_piece(t, g, cur, sums)
        if do_out and not do_attn:
            xn[pl.ds(pl.multiple_of((t - 1) * (R // 2), R // 2), R // 2), :] = xn_new[...]
        if do_out:
            @pl.when(li == 1)
            def _():
                for c in out_copies(t - 1):
                    c.start()

    def out_copies(b):
        r0 = pl.multiple_of(b * R, R)
        h0 = pl.multiple_of(b * (R // 2), R // 2)
        return [pltpu.make_async_copy(xio.at[g, pl.ds(h0, R // 2)].bitcast(BF),
                                      out_hbm.at[pl.ds(r0, R), pl.ds(g * 128, 128)], osems.at[0]) for g in range(G)]

    def layer(li, carry):
        st_f[0] = jnp.full((EP, 1), -jnp.inf, F32)
        st_f[1] = jnp.zeros((EP, 1), F32)
        st_i[...] = jnp.zeros((EP, 1), jnp.int32)
        step(li, -1, True, False, False)
        step(li, 0, True, True, False)
        step(li, 1, True, True, True)

        def steady(t, c):
            step(li, t, True, True, True)
            return c
        lax.fori_loop(2, NB - 1, steady, 0)
        step(li, NB - 1, False, True, True)
        step(li, NB, False, False, True)

        best = st_f[0]
        rmax = jnp.max(best, axis=0, keepdims=True)
        cand = jnp.where(best == rmax, st_i[...], S - 1)
        imin = jnp.min(cand, axis=0, keepdims=True)
        rs = jnp.max(jnp.where(cand == imin, st_f[1], 0.0), axis=0, keepdims=True)
        idx = jnp.clip(jnp.min(cand), 0, S - 1)

        @pl.when(li == 0)
        def _():
            for c in cp_ffn:
                c.wait()

        t0 = pl.multiple_of((idx // 16) * 16, 16)
        th = pl.multiple_of((idx // 16) * 8, 8)
        x2 = [xs[g, pl.ds(t0, 16), :] for g in range(G)]
        xc, _ = _center(x2)
        sel = lax.broadcasted_iota(jnp.int32, (16, 128), 0) == (idx - t0)
        ratio = rs / (1.0 + rs)
        xsel = jnp.concatenate([jnp.where(sel, c * ratio, 0.0) for c in xc], axis=1).astype(BF)
        hs = []
        for j in range(FT):
            gt = jnp.dot(xsel, _up(wg[j]), preferred_element_type=F32)
            ut = jnp.dot(xsel, _up(wu[j]), preferred_element_type=F32)
            hs.append((gt * jax.nn.sigmoid(gt) * ut).astype(BF))
        hh = jnp.concatenate(hs, axis=1)
        gate = jax.nn.sigmoid(rmax)
        x3 = [x2[g] + jnp.where(sel, jnp.dot(hh, _up(wd[g]), preferred_element_type=F32) * gate, 0.0)
              for g in range(G)]

        @pl.when(li == 0)
        def _():
            xc3, v3 = _center(x3)
            rs3 = lax.rsqrt(v3 + EPS)
            for g in range(G):
                xs[g, pl.ds(t0, 16), :] = x3[g]
                xn_b[pl.ds(t0, 16), L(g)] = (xc3[g] * rs3).astype(BF)

        @pl.when(li == 1)
        def _():
            def wait_block(b, c):
                for cp in out_copies(b):
                    cp.wait()
                return c
            lax.fori_loop(0, NB, wait_block, 0)
            for g in range(G):
                xio[g, pl.ds(th, 8), :] = _pk(x3[g])
            cps = [pltpu.make_async_copy(xio.at[g, pl.ds(th, 8)].bitcast(BF),
                                         out_hbm.at[pl.ds(t0, 16), pl.ds(g * 128, 128)], osems.at[0]) for g in range(G)]
            for cp in cps:
                cp.start()
            for cp in cps:
                cp.wait()
        return carry

    lax.fori_loop(0, 2, layer, 0)


@jax.jit
def pallas_interleave_layers__sliding_block__moe_arch_mod__prompt_kernel(
    A_x, A_wqkv, A_wo, B_x, B_w_r, B_w_gate, B_w_up, B_w_down):
    del B_x
    any_spec = pl.BlockSpec(memory_space=pl.ANY)
    out = pl.pallas_call(
        kernel,
        out_shape=jax.ShapeDtypeStruct((S, D), BF),
        in_specs=[any_spec, any_spec, any_spec, pl.BlockSpec(memory_space=pltpu.VMEM), any_spec, any_spec, any_spec],
        out_specs=any_spec,
        scratch_shapes=[
            pltpu.VMEM((G, S // 2, 128), U32),
            pltpu.VMEM((G, S + 32, 128), F32),
            pltpu.VMEM((S // 2, D), U32),
            pltpu.VMEM((3 * G, D // 2, 128), U32),
            pltpu.VMEM((D // 2, D), U32),
            pltpu.VMEM((G, D // 2, 128), U32),
            pltpu.VMEM((FT, D // 2, 128), U32),
            pltpu.VMEM((FT, D // 2, 128), U32),
            pltpu.VMEM((G, F // 2, 128), U32),
            pltpu.VMEM((R // 2, D), U32),
            pltpu.VMEM((R // 2, D), U32),
            pltpu.VMEM((G, 16, 128), F32),
            pltpu.VMEM((2, 16, 1), F32),
            pltpu.VMEM((16, 1), jnp.int32),
            pltpu.SemaphoreType.DMA((XC + 3,)),
            pltpu.SemaphoreType.DMA((1,)),
        ] + [pltpu.VMEM(((S + W) // 2 + 40, 384), U32)] * G + [pltpu.VMEM((128, 512), U32)] * G,
        compiler_params=pltpu.CompilerParams(vmem_limit_bytes=120 * 2**20),
        name="kern",
    )(A_x.reshape(S, D), A_wqkv, A_wo, B_w_r.reshape(G, 128), B_w_gate, B_w_up, B_w_down)
    return out.reshape(1, S, D)
```

```python
import numpy as np
import jax
import jax.numpy as jnp
from jax import lax
import jax.experimental.pallas as pl
import jax.experimental.pallas.tpu as pltpu

S, D, F = 2048, 1024, 3584
DH, W = 32, 256
G = D // 128
FT = F // 128
R = 128
NB = S // R
EP = 16
ROWS = (S + W) // 2
EPS = 1e-5
QSCALE = float(DH ** -0.5 * np.log2(np.e))
NEG = -1e30
BF = jnp.bfloat16
F32 = jnp.float32
U32 = jnp.uint32
NT = (((1,), (1,)), ((), ()))
SPREAD = 180
LAG = 8


def _up(u):
    return pltpu.bitcast(u, BF)


def _L(g):
    return slice(g * 128, (g + 1) * 128)


def _ds(start, size):
    return pl.ds(start if isinstance(start, int) else pl.multiple_of(start, size), size)


def _rowsum(parts):
    s = parts[0]
    for p in parts[1:]:
        s = s + p
    return jnp.sum(s, axis=-1, keepdims=True)


def _center(parts):
    m = _rowsum(parts) * (1.0 / D)
    xc = [p - m for p in parts]
    v = _rowsum([c * c for c in xc]) * (1.0 / D)
    return m, xc, v


def kernel(x_hbm, wqkv_hbm, wo_hbm, wr_ref, wg_hbm, wu_hbm, wd_hbm, out_hbm,
           xin, xout, xs, xn0, xn_new, xn_cur, wqkv, wo, wg, wu, wd, o_s, x1_s, ln_s, wr_s, st_f, st_i,
           xsem, wsem, fsem, osem, *grp):
    qkv_s, p_s = grp[:G], grp[G:]
    qkv_b = [r.bitcast(BF) for r in qkv_s]
    p_b = [r.bitcast(BF) for r in p_s]

    def col_copy(src, dst, j, sem):
        return pltpu.make_async_copy(src.at[:, _ds(j * 128, 128)], dst.at[j].bitcast(BF), sem)

    def x_copy(r0, n, sem):
        return [pltpu.make_async_copy(x_hbm.at[pl.ds(r0, n), pl.ds(j * 128, 128)],
                                      xin.at[j, pl.ds(r0 // 2, n // 2)].bitcast(BF), sem) for j in range(G)]

    def out_copies(r0, n):
        return [pltpu.make_async_copy(xout.at[g, _ds(r0 // 2, n // 2)].bitcast(BF),
                                      out_hbm.at[_ds(r0, n), pl.ds(g * 128, 128)], osem) for g in range(G)]

    cp_x = [x_copy(0, 3 * R, xsem.at[0]), x_copy(3 * R, 2 * R, xsem.at[1]), x_copy(5 * R, S - 5 * R, xsem.at[2])]
    cp_w = [col_copy(wqkv_hbm, wqkv, j, wsem.at[j]) for j in range(3 * G)]
    cp_wo = [col_copy(wo_hbm, wo, j, wsem.at[3 * G]) for j in range(G)]
    KVQ = (2, 1, 0)
    w_grp = [[cp_w[c * G + g] for c in KVQ] for g in range(G)]
    for c in cp_x[0] + w_grp[0]:
        c.start()

    def ffn_copies(act):
        def gate_up(j, c):
            act(col_copy(wg_hbm, wg, j, fsem))
            act(col_copy(wu_hbm, wu, j, fsem))
            return c

        def down(j, c):
            act(col_copy(wd_hbm, wd, j, fsem))
            return c
        lax.fori_loop(0, FT, gate_up, 0)
        lax.fori_loop(0, G, down, 0)

    for g in range(G):
        qkv_s[g][ROWS + 32:ROWS + 40, 0:128] = jnp.zeros((8, 128), U32)
        wr_s[g] = jnp.broadcast_to(wr_ref[g:g + 1, :].astype(F32), (EP, 128))

    tri = lax.broadcasted_iota(jnp.int32, (32, 128), 0) > (lax.broadcasted_iota(jnp.int32, (32, 128), 1) & 31)
    lane = lax.broadcasted_iota(jnp.int32, (16, 128), 1)
    row = lax.broadcasted_iota(jnp.int32, (16, 128), 0)
    u0 = jnp.zeros((16, 128), U32)
    tri_p = (jnp.where(2 * row > (lane & 31), np.uint32(0x0000FFFF), u0)
             | jnp.where(2 * row + 1 > (lane & 31), np.uint32(0xFFFF0000), u0))
    head_of_lane = lane // DH
    odd = (lane & 32) != 0
    upper = (lane & 64) != 0

    def rotate4(ts, zero):
        n = zero.shape[0]

        def sel(m, a, b):
            if a is None and b is None:
                return None
            return jnp.where(m[0:n], zero if a is None else a, zero if b is None else b)
        a = [sel(odd, ts[(1 - k) % 4], ts[-k % 4]) for k in range(4)]
        return [sel(upper, a[(h - 2) % 4], a[h]) for h in range(4)]

    def resid(first, g, r0):
        if first is False:
            return xs[g, _ds(r0, 16), :]
        x = _up(xin[g, _ds(r0 // 2, 8), :]).astype(F32)
        return x if first is True else jnp.where(first, x, xs[g, _ds(r0, 16), :])

    def wide(col):
        return jnp.broadcast_to(col[0:8] + col[8:16], (8, 128))

    def ln_items(load, dst, d0):
        m = _rowsum([load(g) for g in range(G)]) * (1.0 / D)
        yield wide(m)
        xc = [load(g) - m for g in range(G)]
        ss = _rowsum([c * c for c in xc])
        yield wide(ss)
        rs = lax.rsqrt(ss * (1.0 / D) + EPS)
        yield wide(rs)
        for g in range(G):
            y = (load(g) - m) * rs
            dst.bitcast(BF)[d0:d0 + EP, _L(g)] = y.astype(BF)
            if g % 4 == 3:
                yield y[8:16]

    def qkv_piece(src, b, g, col, between=None):
        y = jnp.dot(_up(src[...]), _up(wqkv[col * G + g]), preferred_element_type=F32)
        if between is not None:
            between()
        if col == 0:
            y = y * QSCALE
        if col == 2:
            y = y.astype(BF)
            y = jnp.concatenate([y[i:i + R].T for i in range(0, y.shape[0], R)], axis=0)
        for i in range(y.shape[0] // 16):
            qkv_b[g][_ds((W if col else 0) + b * R + i * 16, 16), _L(col)] = y[i * 16:(i + 1) * 16].astype(BF)
            yield

    def o_piece(first, b, g, src, dst, ln_block=None):
        y = jnp.dot(_up(src[...]), _up(wo[g]), preferred_element_type=F32)
        for i in range(R // 16):
            dst[g, i * 16:(i + 1) * 16, :] = resid(first, g, b * R + i * 16) + y[i * 16:(i + 1) * 16]
            if ln_block is not None:
                ln_s[g, i * 16:(i + 1) * 16, :] = resid(first, g, ln_block * R + i * 16)
            yield

    def epi_items(b, j, src):
        r0 = b * R + j * EP
        load = lambda g: src[g, j * EP:(j + 1) * EP, :]
        m = _rowsum([load(g) for g in range(G)]) * (1.0 / D)
        yield wide(m)
        xc = [load(g) - m for g in range(G)]
        ss = _rowsum([c * c for c in xc])
        yield wide(ss)
        r = _rowsum([(load(g) - m) * wr_s[g] for g in range(G)])
        yield wide(r)
        rs = lax.rsqrt(ss * (1.0 / D) + EPS)
        r = r * rs
        take = r > st_f[0]
        st_f[0] = jnp.where(take, r, st_f[0])
        st_f[1] = jnp.where(take, rs, st_f[1])
        st_i[...] = jnp.where(take, lax.broadcasted_iota(jnp.int32, (EP, 1), 0) + r0, st_i[...])
        yield wide(r)
        for g in range(G):
            x = load(g)
            x2 = x + (x - m) * rs
            xs[g, _ds(r0, EP), :] = x2
            packed = pltpu.bitcast(x2.astype(BF), U32)
            xout[g, _ds(r0 // 2, EP // 2), :] = packed
            if g % 2 == 1:
                yield pltpu.bitcast(packed, F32)

    def epi_piece(b, j, src):
        drain(epi_items(b, j, src))

    def qk_piece(b, g):
        res = []
        for c in range(4):
            q = qkv_s[g][_ds(b * 64 + c * 16, 16), _L(0)]
            w = _up(jnp.concatenate([jnp.where(head_of_lane == (l - c) % 4, q, u0) for l in range(4)], axis=0))
            skip = max(0, 8 - 4 * b - c) if isinstance(b, int) else 0
            k0 = b * 64 + 16 * (c + skip)
            kk = _up(qkv_s[g][pl.ds(k0 if isinstance(k0, int) else pl.multiple_of(k0, 16), 16 * (9 - skip)), _L(1)])
            sc = lax.dot_general(kk, w, NT, preferred_element_type=F32)
            e = jnp.where(tri, NEG if skip else sc[0:32], sc[-32:])
            mid = sc[(0 if skip else 32):-32]
            t = jnp.concatenate([mid, e], axis=0) if mid.shape[0] else e
            res.append((t, jnp.max(t, axis=0, keepdims=True)))
        return res

    def exp_work(g, sc, get_max, sums, off=0):
        for i, (t, _) in enumerate(sc):
            acc = None
            for u in range(t.shape[0] // 16):
                m = get_max(i)
                p = jnp.exp2(t[u * 16:(u + 1) * 16] - jnp.concatenate([m, m], axis=0))
                p_b[g][2 * off + u * 16:2 * off + (u + 1) * 16, _L(i)] = p.astype(BF)
                p = p[0:8] + p[8:16]
                acc = p if acc is None else acc + p
                yield
            sums.append(jnp.sum(acc, axis=0, keepdims=True))

    def pv_piece(b, g, sc, sums, dst, d0, off=0):
        def chunk(c, j):
            n = sc[c][0].shape[0] // 32
            if j < 0 or j > 8 or (n < 8 and j < 9 - n):
                return None
            if j in (0, 8):
                pe = p_s[g][pl.ds(off + 16 * (n - 1), 16), _L(c)]
                return pe & tri_p if j == 0 else pe & ~tri_p
            return p_s[g][pl.ds(off + 16 * (j - 9 + n), 16), _L(c)]
        outs = [None] * 4
        for kt in range(max(0, 2 - b) if isinstance(b, int) else 0, 3):
            ps = [rotate4([chunk(c, pos - c) for c in range(4)], u0) for pos in range(4 * kt, 4 * kt + 4)]
            for h in range(4):
                p = _up(jnp.concatenate([x[h] for x in ps], axis=0))
                vt = _up(qkv_s[g][_ds((b + kt) * 64 + h * 16, 16), _L(2)])
                o = jnp.dot(vt, p, preferred_element_type=F32)
                outs[h] = o if outs[h] is None else outs[h] + o
        inv = rotate4([1.0 / s for s in sums], sums[0])
        outs = [outs[h] * inv[h] for h in range(4)]
        outs = [o if h == 0 else pltpu.roll(o, 128 - 32 * h, axis=1) for h, o in enumerate(outs)]
        dst.bitcast(BF)[_ds(d0, R), _L(g)] = jnp.concatenate(outs, axis=0).astype(BF).T

    def drain(gen):
        for _ in gen:
            pass

    def paced(pieces, works, after=None):
        nwork = sum(n for n, _ in works)
        work = (None for _, w in works for _ in w)
        nch, done, ch = len(pieces) * (R // 16), 0, 0
        for pi, pc in enumerate(pieces):
            for _ in pc:
                ch += 1
                while done < nwork * ch // nch:
                    next(work)
                    done += 1
                if after is not None:
                    after()
        drain(work)

    def softmax(li, g, sc, via, off=0):
        mx = [jnp.broadcast_to(m, (8, 128)) for _, m in sc]
        sums = []
        if via is None:
            get_max = lambda i: mx[i]
        elif isinstance(via, int):
            idx = lambda i: (_ds(ROWS + 40 + 32 * li + 8 * i, 8), _L(1 if off else 0))
            for i in range(4):
                qkv_s[via][idx(i)] = pltpu.bitcast(mx[i], U32)
            get_max = lambda i: pltpu.bitcast(qkv_s[via][idx(i)], F32)
        else:
            idx = lambda i: (G - 1, _ds(R + 32 * li + 8 * i, 8), slice(None))
            for i in range(4):
                via[idx(i)] = mx[i]
            get_max = lambda i: via[idx(i)]
        return (sum(x.shape[0] // 16 for x, _ in sc), exp_work(g, sc, get_max, sums, off)), sums

    def prologue(li):
        first = li == 0

        def sync(wait, start):
            @pl.when(first)
            def _():
                for c in wait:
                    c.wait()
                for c in start:
                    c.start()

        def ln_block(b, dst, d0, js=range(R // EP)):
            for j in js:
                x = [resid(first, g, b * R + j * EP) for g in range(G)]
                drain(ln_items(lambda g: x[g], dst, d0 + j * EP))

        plan = {0: (w_grp[0], w_grp[2]), 1: (w_grp[1], w_grp[3] + w_grp[4]), 2: (w_grp[2], w_grp[5]),
                3: (w_grp[3] + w_grp[4], w_grp[6] + w_grp[7] + cp_x[1]),
                5: (w_grp[5] + w_grp[6] + w_grp[7] + cp_x[1], cp_wo)}
        sync(cp_x[0], w_grp[1])
        ln_block(0, xn0, 0)
        sc = None
        for g in range(G + 1):
            if g in plan:
                sync(*plan[g])
            if g == 0:
                ln_block(1, xn0, R)
                ln_block(2, xn0, 2 * R)
            pieces = [qkv_piece(xn0.at[pl.ds(b * R // 2, R // 2)], b, g, col)
                      for b in range(3) for col in KVQ] if g < G else []
            sm = [softmax(li, g - 1, sc[b], min(g, G - 1), 128 * b) for b in range(2)] if g else []
            if g == G - 1:
                late, pieces = pieces[6:], pieces[:6]
            paced(pieces[:7] if g < G else late[:1], [w for w, _ in sm])
            if g == G:
                drain(late[1])
            cur, sc = sc, [qk_piece(b, g) for b in range(2)] if g < G else None
            for b, (_, sums) in enumerate(sm):
                pv_piece(b, g - 1, cur[b], sums, o_s, b * R, 128 * b)
            for pc in pieces[7:] if g < G else late[2:]:
                drain(pc)
            if g in (5, 6):
                ln_block(3, xn_new, 0, range(4 * (g - 5), 4 * (g - 4)))

    def step(li, t):
        first = li == 0
        ln_block = jnp.minimum(t + 2, NB - 1)
        slot = t % 2
        o_prev = o_s.at[_ds(slot * (R // 2), R // 2)]
        zero = 8 * (li // 2)

        lhs = xn_cur.at[pl.ds(0, R // 2)]
        lhs[...] = xn_new[...]
        drain(o_piece(first, t - 2, 0, o_prev, x1_s, ln_block))
        sc = qk_piece(t, 0)

        def staggered(gens, lead):
            for a, b in zip(gens[0::2], gens[1::2]):
                for x in a:
                    yield x
                    yield next(b)

        def merged():
            e = staggered([epi_items(t - 2, j, x1_s) for j in range(R // EP)], 0)
            n = staggered([ln_items(lambda g, j=j: ln_s[g, j * EP:(j + 1) * EP, :], xn_new, j * EP)
                           for j in range(R // EP)], 0)
            for k in range(104):
                yield (ln_s, n) if k * 5 // 13 != (k + 1) * 5 // 13 else (x1_s, e)
        items = merged()
        pending = []
        count = [0, 0]

        def after(q):
            count[0] += 1
            while pending and pending[0][0] <= count[0]:
                q[_ds(ROWS + zero, 8), _L(0)] = pltpu.bitcast(pending.pop(0)[1], U32)
            if count[1] < 104 * count[0] // SPREAD and count[1] < 104:
                count[1] += 1
                ref, gen = next(items)
                ref[0, _ds(R + 32 * li, 8), :] = pltpu.bitcast(q[ROWS + 32:ROWS + 40, _L(0)], F32)
                pending.append((count[0] + LAG, next(gen)))

        for g in range(G + 1):
            if g == G:
                paced([qkv_piece(lhs, t + 1, G - 1, col,
                                 (lambda: pv_piece(t, G - 1, cur, sums, o_s, slot * R)) if col == KVQ[0] else None)
                       for col in KVQ], [], lambda: after(qkv_s[G - 1]))
                assert count[1] == 104
                break
            if g == 0:
                pieces = [o_piece(first, t - 2, i, o_prev, x1_s, ln_block) for i in range(1, G)]
            else:
                pieces = [qkv_piece(lhs, t + 1, g - 1, col) for col in KVQ]
            work, sums = softmax(li, g, sc, g - 1 if g else x1_s)
            paced(pieces, [work], (lambda: after(qkv_s[g - 1])) if g else None)
            cur = sc
            if g + 1 < G:
                sc = qk_piece(t, g + 1)
                pv_piece(t, g, cur, sums, o_s, slot * R)

    def tail(li):
        first = li == 0
        t = NB - 1
        o13, o14 = o_s.at[pl.ds(R // 2, R // 2)], o_s.at[pl.ds(0, R // 2)]
        fill = ([o_piece(first, t - 2, g, o13, x1_s) for g in range(G)]
                + [o_piece(first, t - 1, g, o14, ln_s) for g in range(G)])
        cuts = (0, 2, 4, 6, 8, 10, 12, 13, 14)

        def pace(ref, tok):
            ref[0, _ds(R + 32 * li, 8), :] = tok

        sc = qk_piece(t, 0)
        for g in range(G):
            work, sums = softmax(li, g, sc, x1_s if g < 4 else ln_s)
            paced(fill[cuts[g]:cuts[g + 1]], [work])
            cur = sc
            if g + 1 < G:
                sc = qk_piece(t, g + 1)
            else:
                drain(fill[14])
            pv_piece(t, g, cur, sums, xn_cur, 0)
            if 3 <= g < 7:
                pace(x1_s, jnp.broadcast_to(sums[0], (8, 128)))
                epi_piece(t - 2, 2 * g - 6, x1_s)
                epi_piece(t - 2, 2 * g - 5, x1_s)
        drain(fill[15])
        for g in range(G):
            epi_piece(t - 1, g, ln_s)
            drain(o_piece(first, t, g, xn_cur.at[pl.ds(0, R // 2)], x1_s))
            pace(ln_s, x1_s[g, R - 8:R, :])
        for j in range(R // EP):
            epi_piece(t, j, x1_s)

    def flush(cond, b, n=1):
        @pl.when(cond)
        def _():
            for c in out_copies(b * R, n * R):
                c.start()

    def layer(li, carry):
        st_f[0] = jnp.full((EP, 1), -jnp.inf, F32)
        st_f[1] = jnp.zeros((EP, 1), F32)
        st_i[...] = jnp.zeros((EP, 1), jnp.int32)
        prologue(li)

        def steady(t, c):
            @pl.when(jnp.logical_and(li == 0, t == 2))
            def _():
                for cp in cp_wo:
                    cp.wait()
                for cp in cp_x[2]:
                    cp.start()

            @pl.when(jnp.logical_and(li == 0, t == 3))
            def _():
                for cp in cp_x[2]:
                    cp.wait()
            flush(jnp.logical_and(li == 1, t >= 3), jnp.maximum(t - 3, 0))

            @pl.when((li == 0) & (t >= 3) & (t < 3 + FT // 4))
            def _():
                for j in range(4):
                    col_copy(wg_hbm, wg, (t - 3) * 4 + j, fsem).start()
                    col_copy(wu_hbm, wu, (t - 3) * 4 + j, fsem).start()

            @pl.when((li == 0) & (t >= 3) & (t < 3 + G))
            def _():
                col_copy(wd_hbm, wd, t - 3, fsem).start()
            step(li, t)
            return c
        lax.fori_loop(2, NB - 1, steady, 0)

        @pl.when(li == 0)
        def _():
            ffn_copies(lambda c: c.wait())

        flush(li == 1, NB - 4)
        tail(li)
        flush(li == 1, NB - 3, 3)

        best = st_f[0]
        rmax = jnp.max(best, axis=0, keepdims=True)
        cand = jnp.where(best == rmax, st_i[...], S - 1)
        imin = jnp.min(cand, axis=0, keepdims=True)
        rs = jnp.max(jnp.where(cand == imin, st_f[1], 0.0), axis=0, keepdims=True)
        idx = jnp.clip(jnp.min(cand), 0, S - 1)

        t0 = (idx // 16) * 16
        x2 = [xs[g, _ds(t0, 16), :] for g in range(G)]
        _, xc, _ = _center(x2)
        sel = lax.broadcasted_iota(jnp.int32, (16, 128), 0) == (idx - t0)
        ratio = rs / (1.0 + rs)
        xsel = jnp.concatenate([jnp.where(sel, c * ratio, 0.0) for c in xc], axis=1).astype(BF)
        hs = []
        for j in range(FT):
            gt = jnp.dot(xsel, _up(wg[j]), preferred_element_type=F32)
            ut = jnp.dot(xsel, _up(wu[j]), preferred_element_type=F32)
            hs.append(gt * jax.nn.sigmoid(gt) * ut)
        hh = jnp.concatenate(hs, axis=1).astype(BF)
        gate = jax.nn.sigmoid(rmax)
        x3 = [x2[g] + jnp.where(sel, jnp.dot(hh, _up(wd[g]), preferred_element_type=F32) * gate, 0.0)
              for g in range(G)]

        for g in range(G):
            xs[g, _ds(t0, 16), :] = x3[g]

        @pl.when(li == 1)
        def _():
            def wait_block(b, c):
                for cp in out_copies(b * R, R):
                    cp.wait()
                return c
            lax.fori_loop(0, NB - 3, wait_block, 0)
            for cp in out_copies((NB - 3) * R, 3 * R):
                cp.wait()
            for g in range(G):
                xout[g, _ds(t0 // 2, 8), :] = pltpu.bitcast(x3[g].astype(BF), U32)
            cps = out_copies(t0, 16)
            for cp in cps:
                cp.start()
            for cp in cps:
                cp.wait()
        return carry

    lax.fori_loop(0, 2, layer, 0)


@jax.jit
def pallas_interleave_layers__sliding_block__moe_arch_mod__prompt_kernel(
    A_x, A_wqkv, A_wo, B_x, B_w_r, B_w_gate, B_w_up, B_w_down):
    del B_x
    any_spec = pl.BlockSpec(memory_space=pl.ANY)
    out = pl.pallas_call(
        kernel,
        out_shape=jax.ShapeDtypeStruct((S, D), BF),
        in_specs=[any_spec, any_spec, any_spec, pl.BlockSpec(memory_space=pltpu.VMEM), any_spec, any_spec, any_spec],
        out_specs=any_spec,
        scratch_shapes=[
            pltpu.VMEM((G, S // 2, 128), U32),
            pltpu.VMEM((G, S // 2, 128), U32),
            pltpu.VMEM((G, S, 128), F32),
            pltpu.VMEM((3 * R // 2, D), U32),
            pltpu.VMEM((R // 2, D), U32),
            pltpu.VMEM((R // 2 + 8, D), U32),
            pltpu.VMEM((3 * G, D // 2, 128), U32),
            pltpu.VMEM((G, D // 2, 128), U32),
            pltpu.VMEM((FT, D // 2, 128), U32),
            pltpu.VMEM((FT, D // 2, 128), U32),
            pltpu.VMEM((G, F // 2, 128), U32),
            pltpu.VMEM((R, D), U32),
            pltpu.VMEM((G, R + 64, 128), F32),
            pltpu.VMEM((G, R + 64, 128), F32),
            pltpu.VMEM((G, EP, 128), F32),
            pltpu.VMEM((2, EP, 1), F32),
            pltpu.VMEM((EP, 1), jnp.int32),
            pltpu.SemaphoreType.DMA((3,)),
            pltpu.SemaphoreType.DMA((3 * G + 1,)),
            pltpu.SemaphoreType.DMA(()),
            pltpu.SemaphoreType.DMA(()),
        ] + [pltpu.VMEM((ROWS + 104, 384), U32)] * G + [pltpu.VMEM((256, 512), U32)] * G,
        compiler_params=pltpu.CompilerParams(vmem_limit_bytes=120 * 2**20, disable_bounds_checks=True),
        name="kern",
    )(A_x.reshape(S, D), A_wqkv, A_wo, B_w_r.reshape(G, 128), B_w_gate, B_w_up, B_w_down)
    return out.reshape(1, S, D)
```

```python
import numpy as np
import jax
import jax.numpy as jnp
from jax import lax
import jax.experimental.pallas as pl
import jax.experimental.pallas.tpu as pltpu

S, D, F = 2048, 1024, 3584
DH, W = 32, 256
G = D // 128
FT = F // 128
R = 128
NB = S // R
EP = 16
ROWS = (S + W) // 2
EPS = 1e-5
QSCALE = float(DH ** -0.5 * np.log2(np.e))
NEG = -1e30
BF = jnp.bfloat16
F32 = jnp.float32
U32 = jnp.uint32
NT = (((1,), (1,)), ((), ()))
import os
SPREAD = int(os.environ.get('SPREAD', 340))
LAG = int(os.environ.get('LAG', 20))
NV = 4
EARLY = int(os.environ.get('EARLY', 0))


def _up(u):
    return pltpu.bitcast(u, BF)


def _L(g):
    return slice(g * 128, (g + 1) * 128)


def _ds(start, size):
    return pl.ds(start if isinstance(start, int) else pl.multiple_of(start, size), size)


def _rowsum(parts):
    s = parts[0]
    for p in parts[1:]:
        s = s + p
    return jnp.sum(s, axis=-1, keepdims=True)


def _center(parts):
    m = _rowsum(parts) * (1.0 / D)
    xc = [p - m for p in parts]
    v = _rowsum([c * c for c in xc]) * (1.0 / D)
    return m, xc, v


def kernel(x_hbm, wqkv_hbm, wo_hbm, wr_hbm, wg_hbm, wu_hbm, wd_hbm, out_hbm,
           xin, xout, xs, xn0, xn_new, xn_cur, wqkv, wo, wg, wu, wd, o_s, x1_s, ln_s, wr_ref, wr_s, st_f, st_i,
           xsem, wsem, fsem, osem, *grp):
    qkv_s, p_s = grp[:G], grp[G:]
    qkv_b = [r.bitcast(BF) for r in qkv_s]
    p_b = [r.bitcast(BF) for r in p_s]

    def col_copy(src, dst, j, sem):
        return pltpu.make_async_copy(src.at[:, _ds(j * 128, 128)], dst.at[j].bitcast(BF), sem)

    def x_copy(r0, n, sem):
        return [pltpu.make_async_copy(x_hbm.at[pl.ds(r0, n), pl.ds(j * 128, 128)],
                                      xin.at[j, pl.ds(r0 // 2, n // 2)].bitcast(BF), sem) for j in range(G)]

    def out_copies(r0, n):
        return [pltpu.make_async_copy(xout.at[g, _ds(r0 // 2, n // 2)].bitcast(BF),
                                      out_hbm.at[_ds(r0, n), pl.ds(g * 128, 128)], osem) for g in range(G)]

    cp_x = [x_copy(0, R, xsem.at[0]), x_copy(3 * R, 2 * R, xsem.at[1]), x_copy(5 * R, S - 5 * R, xsem.at[2]),
            x_copy(R, 2 * R, xsem.at[3]) + [pltpu.make_async_copy(wr_hbm, wr_ref, xsem.at[3])]]
    cp_w = [col_copy(wqkv_hbm, wqkv, j, wsem.at[j]) for j in range(3 * G)]
    cp_wo = [col_copy(wo_hbm, wo, j, wsem.at[3 * G]) for j in range(G)]
    KVQ = (2, 1, 0)
    w_grp = [[cp_w[c * G + g] for c in KVQ] for g in range(G)]
    for c in cp_x[0] + w_grp[0] + cp_x[3]:
        c.start()

    def ffn_copies(act):
        def gate_up(j, c):
            act(col_copy(wg_hbm, wg, j, fsem))
            act(col_copy(wu_hbm, wu, j, fsem))
            return c

        def down(j, c):
            act(col_copy(wd_hbm, wd, j, fsem))
            return c
        lax.fori_loop(0, FT, gate_up, 0)
        lax.fori_loop(0, G, down, 0)

    for g in range(G):
        qkv_s[g][ROWS + 32:ROWS + 40, 0:128] = jnp.zeros((8, 128), U32)

    tri = lax.broadcasted_iota(jnp.int32, (32, 128), 0) > (lax.broadcasted_iota(jnp.int32, (32, 128), 1) & 31)
    lane = lax.broadcasted_iota(jnp.int32, (16, 128), 1)
    row = lax.broadcasted_iota(jnp.int32, (16, 128), 0)
    u0 = jnp.zeros((16, 128), U32)
    tri_p = (jnp.where(2 * row > (lane & 31), np.uint32(0x0000FFFF), u0)
             | jnp.where(2 * row + 1 > (lane & 31), np.uint32(0xFFFF0000), u0))
    head_of_lane = lane // DH
    odd = (lane & 32) != 0
    upper = (lane & 64) != 0

    def rotate4(ts, zero):
        n = zero.shape[0]

        def sel(m, a, b):
            if a is None and b is None:
                return None
            return jnp.where(m[0:n], zero if a is None else a, zero if b is None else b)
        a = [sel(odd, ts[(1 - k) % 4], ts[-k % 4]) for k in range(4)]
        return [sel(upper, a[(h - 2) % 4], a[h]) for h in range(4)]

    def resid(first, g, r0):
        if first is False:
            return xs[g, _ds(r0, 16), :]
        x = _up(xin[g, _ds(r0 // 2, 8), :]).astype(F32)
        return x if first is True else jnp.where(first, x, xs[g, _ds(r0, 16), :])

    def wide(col):
        return jnp.broadcast_to(col[0:8] + col[8:16], (8, 128))

    def ln_items(load, dst, d0):
        m = _rowsum([load(g) for g in range(G)]) * (1.0 / D)
        yield wide(m)
        xc = [load(g) - m for g in range(G)]
        ss = _rowsum([c * c for c in xc])
        yield wide(ss)
        rs = lax.rsqrt(ss * (1.0 / D) + EPS)
        yield wide(rs)
        for g in range(G):
            y = (load(g) - m) * rs
            dst.bitcast(BF)[d0:d0 + EP, _L(g)] = y.astype(BF)
            if g % 4 == 3:
                yield y[8:16]

    CH = 2 * R // 16

    def halves(src, w, j):
        return [jnp.dot(_up(src[:, h * D // 2:(h + 1) * D // 2]), _up(w[j, h * D // 4:(h + 1) * D // 4, :]),
                        preferred_element_type=F32) for h in range(2)]

    def qkv_pieces(zero, src, b, g, between=None):
        def mark(y):
            if zero is None:
                return
            qkv_s[g][_ds(ROWS + 8 + zero, 8), _L(0)] = pltpu.bitcast(y[8:16], U32)

        def put(col, i, y):
            qkv_b[g][_ds((W if col else 0) + b * R + i * 16, 16), _L(col)] = y.astype(BF)
        vt = []

        def piece(col):
            y0, y1 = halves(src, wqkv, col * G + g)
            if col == 2 and between is not None:
                between()
            rows = [slice(i * 16, (i + 1) * 16) for i in range(R // 16)]
            for r in rows:
                mark(y0[r])
                yield
            y = y0 + y1
            if col == 2:
                vt.append(y.astype(BF).T)
            for i, r in enumerate(rows):
                if col == 2:
                    mark(y[r])
                else:
                    put(col, i, y[r] * QSCALE if col == 0 else y[r])
                if col == 1 and i == len(rows) - 1:
                    for k, rk in enumerate(rows):
                        put(2, k, vt[0][rk])
                yield
        return [piece(col) for col in KVQ]

    def o_piece(first, b, g, src, dst, ln_block=None):
        y0, y1 = halves(src, wo, g)
        rows = [slice(i * 16, (i + 1) * 16) for i in range(R // 16)]
        for i, r in enumerate(rows):
            dst[g, r, :] = resid(first, g, b * R + i * 16) + y0[r]
            yield
        for i, r in enumerate(rows):
            dst[g, r, :] = dst[g, r, :] + y1[r]
            if ln_block is not None:
                ln_s[g, r, :] = resid(first, g, ln_block * R + i * 16)
            yield

    def epi_items(b, j, src):
        r0 = b * R + j * EP
        load = lambda g: src[g, j * EP:(j + 1) * EP, :]
        m = _rowsum([load(g) for g in range(G)]) * (1.0 / D)
        yield wide(m)
        xc = [load(g) - m for g in range(G)]
        ss = _rowsum([c * c for c in xc])
        yield wide(ss)
        r = _rowsum([(load(g) - m) * wr_s[g] for g in range(G)])
        yield wide(r)
        rs = lax.rsqrt(ss * (1.0 / D) + EPS)
        r = r * rs
        take = r > st_f[0]
        st_f[0] = jnp.where(take, r, st_f[0])
        st_f[1] = jnp.where(take, rs, st_f[1])
        st_i[...] = jnp.where(take, lax.broadcasted_iota(jnp.int32, (EP, 1), 0) + r0, st_i[...])
        yield wide(r)
        for g in range(G):
            x = load(g)
            x2 = x + (x - m) * rs
            xs[g, _ds(r0, EP), :] = x2
            packed = pltpu.bitcast(x2.astype(BF), U32)
            xout[g, _ds(r0 // 2, EP // 2), :] = packed
            if g % 2 == 1:
                yield pltpu.bitcast(packed, F32)

    def epi_piece(b, j, src):
        drain(epi_items(b, j, src))

    def qk_piece(b, g):
        res = []
        for c in range(4):
            q = qkv_s[g][_ds(b * 64 + c * 16, 16), _L(0)]
            w = _up(jnp.concatenate([jnp.where(head_of_lane == (l - c) % 4, q, u0) for l in range(4)], axis=0))
            skip = max(0, 8 - 4 * b - c) if isinstance(b, int) else 0
            k0 = b * 64 + 16 * (c + skip)
            kk = _up(qkv_s[g][pl.ds(k0 if isinstance(k0, int) else pl.multiple_of(k0, 16), 16 * (9 - skip)), _L(1)])
            sc = lax.dot_general(kk, w, NT, preferred_element_type=F32)
            e = jnp.where(tri, NEG if skip else sc[0:32], sc[-32:])
            mid = sc[(0 if skip else 32):-32]
            t = jnp.concatenate([mid, e], axis=0) if mid.shape[0] else e
            res.append((t, jnp.max(t, axis=0, keepdims=True)))
        return res

    def exp_work(g, sc, get_max, sums, off=0):
        for i, (t, _) in enumerate(sc):
            acc = None
            for u in range(t.shape[0] // 16):
                m = get_max(i)
                p = jnp.exp2(t[u * 16:(u + 1) * 16] - jnp.concatenate([m, m], axis=0))
                p_b[g][2 * off + u * 16:2 * off + (u + 1) * 16, _L(i)] = p.astype(BF)
                p = p[0:8] + p[8:16]
                acc = p if acc is None else acc + p
                yield
            sums.append(jnp.sum(acc, axis=0, keepdims=True))

    def pv_piece(b, g, sc, sums, dst, d0, off=0):
        def chunk(c, j):
            n = sc[c][0].shape[0] // 32
            if j < 0 or j > 8 or (n < 8 and j < 9 - n):
                return None
            if j in (0, 8):
                pe = p_s[g][pl.ds(off + 16 * (n - 1), 16), _L(c)]
                return pe & tri_p if j == 0 else pe & ~tri_p
            return p_s[g][pl.ds(off + 16 * (j - 9 + n), 16), _L(c)]
        outs = [None] * 4
        for kt in range(max(0, 2 - b) if isinstance(b, int) else 0, 3):
            ps = [rotate4([chunk(c, pos - c) for c in range(4)], u0) for pos in range(4 * kt, 4 * kt + 4)]
            for h in range(4):
                p = _up(jnp.concatenate([x[h] for x in ps], axis=0))
                vt = _up(qkv_s[g][_ds((b + kt) * 64 + h * 16, 16), _L(2)])
                o = jnp.dot(vt, p, preferred_element_type=F32)
                outs[h] = o if outs[h] is None else outs[h] + o
        inv = rotate4([1.0 / s for s in sums], sums[0])
        outs = [outs[h] * inv[h] for h in range(4)]
        outs = [o if h == 0 else pltpu.roll(o, 128 - 32 * h, axis=1) for h, o in enumerate(outs)]
        dst.bitcast(BF)[_ds(d0, R), _L(g)] = jnp.concatenate(outs, axis=0).astype(BF).T

    def drain(gen):
        for _ in gen:
            pass

    def paced(pieces, works, after=None):
        nwork = sum(n for n, _ in works)
        work = (None for _, w in works for _ in w)
        nch, done, ch = len(pieces) * CH - EARLY, 0, 0
        for pi, pc in enumerate(pieces):
            for _ in pc:
                ch += 1
                while done < min(nwork, nwork * ch // nch):
                    next(work)
                    done += 1
                if after is not None:
                    after()
        drain(work)

    def softmax(li, g, sc, via, off=0):
        mx = [jnp.broadcast_to(m, (8, 128)) for _, m in sc]
        sums = []
        if via is None:
            get_max = lambda i: mx[i]
        elif isinstance(via, int):
            idx = lambda i: (_ds(ROWS + 40 + 32 * li + 8 * i, 8), _L(1 if off else 0))
            for i in range(4):
                qkv_s[via][idx(i)] = pltpu.bitcast(mx[i], U32)
            get_max = lambda i: pltpu.bitcast(qkv_s[via][idx(i)], F32)
        else:
            idx = lambda i: (G - 1, _ds(R + 32 * li + 8 * i, 8), slice(None))
            for i in range(4):
                via[idx(i)] = mx[i]
            get_max = lambda i: via[idx(i)]
        return (sum(x.shape[0] // 16 for x, _ in sc), exp_work(g, sc, get_max, sums, off)), sums

    def prologue(li):
        first = li == 0

        def sync(wait, start):
            @pl.when(first)
            def _():
                for c in wait:
                    c.wait()
                for c in start:
                    c.start()

        def ln_block(b, dst, d0, js=range(R // EP)):
            for j in js:
                x = [resid(first, g, b * R + j * EP) for g in range(G)]
                drain(ln_items(lambda g: x[g], dst, d0 + j * EP))

        plan = {0: (w_grp[0] + cp_x[3], w_grp[2]), 1: (w_grp[1], w_grp[3] + w_grp[4]), 2: (w_grp[2], w_grp[5]),
                3: (w_grp[3] + w_grp[4], w_grp[6] + w_grp[7] + cp_x[1]),
                5: (w_grp[5] + w_grp[6] + w_grp[7] + cp_x[1], cp_wo)}
        sync(cp_x[0], w_grp[1])
        ln_block(0, xn0, 0)
        sc = None
        for g in range(G + 1):
            if g in plan:
                sync(*plan[g])
            if g == 0:
                ln_block(1, xn0, R)
                ln_block(2, xn0, 2 * R)
            if g == 1:
                for i in range(G):
                    wr_s[i] = jnp.broadcast_to(wr_ref[i:i + 1, :].astype(F32), (EP, 128))
            pieces = [pc for b in range(3)
                      for pc in qkv_pieces(8 * (li // 2) if (0 < g and b < 2) or g == G - 1 else None, xn0.at[pl.ds(b * R // 2, R // 2)], b, g)] if g < G else []
            sm = [softmax(li, g - 1, sc[b], min(g, G - 1), 128 * b) for b in range(2)] if g else []
            if g == G - 1:
                late, pieces = pieces[6:], pieces[:6]
            paced(pieces[:5] if g < G else late[:1], [w for w, _ in sm])
            for pc in pieces[5:7] if g < G else late[1:2]:
                drain(pc)
            cur, sc = sc, [qk_piece(b, g) for b in range(2)] if g < G else None
            for b, (_, sums) in enumerate(sm):
                pv_piece(b, g - 1, cur[b], sums, o_s, b * R, 128 * b)
            for pc in pieces[7:] if g < G else late[2:]:
                drain(pc)
            if g in (5, 6):
                ln_block(3, xn_new, 0, range(4 * (g - 5), 4 * (g - 4)))

    def step(li, t):
        first = li == 0
        ln_block = jnp.minimum(t + 2, NB - 1)
        slot = t % 2
        o_prev = o_s.at[_ds(slot * (R // 2), R // 2)]
        zero = 8 * (li // 2)

        lhs = xn_cur.at[pl.ds(0, R // 2)]

        def o_and_copy(i):
            lhs[:, _L(i)] = xn_new[:, _L(i)]
            x1_s[1, _ds(R + 32 * li, 8), :] = pltpu.bitcast(xn_cur[_ds(zero, 8), _L(i)], F32)
            if i == 1:
                @pl.when(first & (t == 2))
                def _():
                    for cp in cp_x[2]:
                        cp.start()
            if i == 3:
                @pl.when(first & (t >= 3) & (t < 3 + FT // 4))
                def _():
                    for j in range(4):
                        col_copy(wg_hbm, wg, (t - 3) * 4 + j, fsem).start()
                        col_copy(wu_hbm, wu, (t - 3) * 4 + j, fsem).start()

                @pl.when(first & (t >= 3) & (t < 3 + G))
                def _():
                    col_copy(wd_hbm, wd, t - 3, fsem).start()
            if i == 2:
                flush((li == 1) & (t >= 3), jnp.maximum(t - 3, 0))
            yield from o_piece(first, t - 2, i, o_prev, x1_s, ln_block)
        drain(o_and_copy(0))
        sc = qk_piece(t, 0)

        def staggered(gens, lead):
            for a, b in zip(gens[0::2], gens[1::2]):
                for x in a:
                    yield x
                    yield next(b)

        def merged():
            e = staggered([epi_items(t - 2, j, x1_s) for j in range(R // EP)], 0)
            n = staggered([ln_items(lambda g, j=j: ln_s[g, j * EP:(j + 1) * EP, :], xn_new, j * EP)
                           for j in range(R // EP)], 0)
            for k in range(104):
                yield (ln_s, n) if k * 5 // 13 != (k + 1) * 5 // 13 else (x1_s, e)
        items = merged()
        pending = []
        count = [0, 0]

        def after(q):
            count[0] += 1
            while pending and pending[0][0] <= count[0]:
                q[_ds(ROWS + zero, 8), _L(0)] = pltpu.bitcast(pending.pop(0)[1], U32)
            if count[1] < 104 * count[0] // SPREAD and count[1] < 104:
                count[1] += 1
                ref, gen = next(items)
                ref[0, _ds(R + 32 * li, 8), :] = pltpu.bitcast(q[ROWS + 32:ROWS + 40, _L(0)], F32)
                pending.append((count[0] + LAG, next(gen)))

        for g in range(G + 1):
            if g == G:
                paced(qkv_pieces(zero, lhs, t + 1, G - 1, lambda: pv_piece(t, G - 1, cur, sums, o_s, slot * R)),
                      [], lambda: after(qkv_s[G - 1]))
                assert count[1] == 104
                break
            if g == 0:
                pieces = [o_and_copy(i) for i in range(1, G)]
            else:
                pieces = qkv_pieces(zero, lhs, t + 1, g - 1)
            work, sums = softmax(li, g, sc, g - 1 if g else x1_s)
            paced(pieces, [work], (lambda: after(qkv_s[g - 1])) if g else None)
            cur = sc
            if g + 1 < G:
                sc = qk_piece(t, g + 1)
                pv_piece(t, g, cur, sums, o_s, slot * R)

    def tail(li):
        first = li == 0
        t = NB - 1
        o13, o14 = o_s.at[pl.ds(R // 2, R // 2)], o_s.at[pl.ds(0, R // 2)]
        fill = ([o_piece(first, t - 2, g, o13, x1_s) for g in range(G)]
                + [o_piece(first, t - 1, g, o14, ln_s) for g in range(G)])
        cuts = (0, 2, 4, 6, 8, 10, 12, 13, 14)

        def pace(ref, tok):
            ref[0, _ds(R + 32 * li, 8), :] = tok

        sc = qk_piece(t, 0)
        for g in range(G):
            work, sums = softmax(li, g, sc, x1_s if g < 4 else ln_s)
            paced(fill[cuts[g]:cuts[g + 1]], [work])
            cur = sc
            if g + 1 < G:
                sc = qk_piece(t, g + 1)
            else:
                drain(fill[14])
            pv_piece(t, g, cur, sums, xn_cur, 0)
            if 3 <= g < 7:
                pace(x1_s, jnp.broadcast_to(sums[0], (8, 128)))
                epi_piece(t - 2, 2 * g - 6, x1_s)
                epi_piece(t - 2, 2 * g - 5, x1_s)
        drain(fill[15])
        for g in range(G):
            epi_piece(t - 1, g, ln_s)
            drain(o_piece(first, t, g, xn_cur.at[pl.ds(0, R // 2)], x1_s))
            pace(ln_s, x1_s[g, R - 8:R, :])
        for j in range(R // EP):
            epi_piece(t, j, x1_s)

    def flush(cond, b, n=1):
        @pl.when(cond)
        def _():
            for c in out_copies(b * R, n * R):
                c.start()

    def layer(li, carry):
        st_f[0] = jnp.full((EP, 1), -jnp.inf, F32)
        st_f[1] = jnp.zeros((EP, 1), F32)
        st_i[...] = jnp.zeros((EP, 1), jnp.int32)
        prologue(li)

        def steady(t, c):
            for when, cps in ((2, cp_wo), (3, cp_x[2])):
                @pl.when((li == 0) & (t == when))
                def _():
                    for cp in cps:
                        cp.wait()
            step(li, t)
            return c
        lax.fori_loop(2, NB - 1, steady, 0)

        @pl.when(li == 0)
        def _():
            ffn_copies(lambda c: c.wait())

        flush(li == 1, NB - 4)
        tail(li)
        flush(li == 1, NB - 3, 3)

        best = st_f[0]
        rmax = jnp.max(best, axis=0, keepdims=True)
        cand = jnp.where(best == rmax, st_i[...], S - 1)
        imin = jnp.min(cand, axis=0, keepdims=True)
        rs = jnp.max(jnp.where(cand == imin, st_f[1], 0.0), axis=0, keepdims=True)
        idx = jnp.clip(jnp.min(cand), 0, S - 1)

        t0 = (idx // 16) * 16
        _, xc, _ = _center([xs[g, pl.ds(idx, 1), :] for g in range(G)])
        xrow = [(c * (rs / (1.0 + rs))).astype(BF).astype(F32) for c in xc]
        xsel = jnp.concatenate([jnp.broadcast_to(x, (16, 128)) for x in xrow], axis=1).astype(BF)
        for g in range(G):
            ln_s[g, 0:128, :] = jnp.broadcast_to(xrow[g], (128, 128)).T

        def vpu_matvec(tiles):
            acc = [None] * len(tiles)
            for k in range(D // 16):
                even = ln_s[k // 8, pl.ds((k % 8) * 16, 8, stride=2), :]
                odd_ = ln_s[k // 8, pl.ds((k % 8) * 16 + 1, 8, stride=2), :]
                for i, (w, j) in enumerate(tiles):
                    u = w[j, k * 8:(k + 1) * 8, :]
                    p = (pltpu.bitcast(u << 16, F32) * even
                         + pltpu.bitcast(u & np.uint32(0xFFFF0000), F32) * odd_)
                    acc[i] = p if acc[i] is None else acc[i] + p
            return [jnp.sum(a, axis=0, keepdims=True) for a in acc]

        y = [None] * G

        def down(j, gt, ut):
            h = jnp.broadcast_to(gt * jax.nn.sigmoid(gt) * ut, (16, 128)).astype(BF)
            for g in range(G):
                p = jnp.dot(h, _up(wd[g, j * 64:(j + 1) * 64, :]), preferred_element_type=F32)[0:8]
                y[g] = p if y[g] is None else y[g] + p

        ready = []
        for j0 in range(0, FT, 7):
            for j in range(j0, j0 + 7 - NV):
                ready.append((j, jnp.dot(xsel, _up(wg[j]), preferred_element_type=F32)[0:1],
                              jnp.dot(xsel, _up(wu[j]), preferred_element_type=F32)[0:1]))
            while ready:
                down(*ready.pop(0))
            for j in range(j0 + 7 - NV, j0 + 7, 2):
                r = vpu_matvec([(w, jj) for jj in (j, j + 1) for w in (wg, wu)])
                ready += [(j, r[0], r[1]), (j + 1, r[2], r[3])]
        while ready:
            down(*ready.pop(0))
        gate = jax.nn.sigmoid(rmax)
        sel = lax.broadcasted_iota(jnp.int32, (16, 128), 0) == (idx - t0)
        x3 = [xs[g, _ds(t0, 16), :] + jnp.where(sel, y[g][0:1] * gate, 0.0) for g in range(G)]

        for g in range(G):
            xs[g, _ds(t0, 16), :] = x3[g]

        @pl.when(li == 1)
        def _():
            def wait_block(b, c):
                for cp in out_copies(b * R, R):
                    cp.wait()
                return c
            lax.fori_loop(0, NB - 3, wait_block, 0)
            for cp in out_copies((NB - 3) * R, 3 * R):
                cp.wait()
            for g in range(G):
                xout[g, _ds(t0 // 2, 8), :] = pltpu.bitcast(x3[g].astype(BF), U32)
            cps = out_copies(t0, 16)
            for cp in cps:
                cp.start()
            for cp in cps:
                cp.wait()
        return carry

    lax.fori_loop(0, 2, layer, 0)


@jax.jit
def pallas_interleave_layers__sliding_block__moe_arch_mod__prompt_kernel(
    A_x, A_wqkv, A_wo, B_x, B_w_r, B_w_gate, B_w_up, B_w_down):
    del B_x
    any_spec = pl.BlockSpec(memory_space=pl.ANY)
    out = pl.pallas_call(
        kernel,
        out_shape=jax.ShapeDtypeStruct((S, D), BF),
        in_specs=[any_spec, any_spec, any_spec, any_spec, any_spec, any_spec, any_spec],
        out_specs=any_spec,
        scratch_shapes=[
            pltpu.VMEM((G, S // 2, 128), U32),
            pltpu.VMEM((G, S // 2, 128), U32),
            pltpu.VMEM((G, S, 128), F32),
            pltpu.VMEM((3 * R // 2, D), U32),
            pltpu.VMEM((R // 2, D), U32),
            pltpu.VMEM((R // 2 + 8, D), U32),
            pltpu.VMEM((3 * G, D // 2, 128), U32),
            pltpu.VMEM((G, D // 2, 128), U32),
            pltpu.VMEM((FT, D // 2, 128), U32),
            pltpu.VMEM((FT, D // 2, 128), U32),
            pltpu.VMEM((G, F // 2, 128), U32),
            pltpu.VMEM((R, D), U32),
            pltpu.VMEM((G, R + 64, 128), F32),
            pltpu.VMEM((G, R + 64, 128), F32),
            pltpu.VMEM((G, 128), BF),
            pltpu.VMEM((G, EP, 128), F32),
            pltpu.VMEM((2, EP, 1), F32),
            pltpu.VMEM((EP, 1), jnp.int32),
            pltpu.SemaphoreType.DMA((4,)),
            pltpu.SemaphoreType.DMA((3 * G + 1,)),
            pltpu.SemaphoreType.DMA(()),
            pltpu.SemaphoreType.DMA(()),
        ] + [pltpu.VMEM((ROWS + 104, 384), U32)] * G + [pltpu.VMEM((256, 512), U32)] * G,
        compiler_params=pltpu.CompilerParams(vmem_limit_bytes=120 * 2**20, disable_bounds_checks=True),
        name="kern",
    )(A_x.reshape(S, D), A_wqkv, A_wo, B_w_r.reshape(G, 128), B_w_gate, B_w_up, B_w_down)
    return out.reshape(1, S, D)
```

```python
import numpy as np
import jax
import jax.numpy as jnp
from jax import lax
import jax.experimental.pallas as pl
import jax.experimental.pallas.tpu as pltpu

S, D, F = 2048, 1024, 3584
DH, W = 32, 256
G = D // 128
FT = F // 128
R = 128
NB = S // R
EP = 16
ROWS = (S + W) // 2
CH = 2 * R // 16
EPS = 1e-5
QSCALE = float(DH ** -0.5 * np.log2(np.e))
NEG = -1e30
BF, F32, U32 = jnp.bfloat16, jnp.float32, jnp.uint32
NT = (((1,), (1,)), ((), ()))
VKQ = (2, 1, 0)
N_LN, N_EPI = 5 * R // EP, 8 * R // EP
SPREAD, LAG = 330, 24
NV = 4


def _up(u):
    return pltpu.bitcast(u, BF)


def _L(g):
    return slice(g * 128, (g + 1) * 128)


def _ds(start, size):
    return pl.ds(start if isinstance(start, int) else pl.multiple_of(start, size), size)


def _rowsum(parts):
    s = parts[0]
    for p in parts[1:]:
        s = s + p
    return jnp.sum(s, axis=-1, keepdims=True)


def _drain(gen):
    for _ in gen:
        pass


def _kernel(x_hbm, wqkv_hbm, wo_hbm, wr_hbm, wg_hbm, wu_hbm, wd_hbm, out_hbm,
            xin, xout, xs, xn0, xn_new, xn_cur, wqkv, wo, wg, wu, wd, o_s, x1_s, ln_s,
            wr_in, wr_s, st_f, st_i, xsem, wsem, fsem, osem, *grp):
    qkv_s, p_s = grp[:G], grp[G:]
    qkv_b = [r.bitcast(BF) for r in qkv_s]
    p_b = [r.bitcast(BF) for r in p_s]

    def col_copy(src, dst, j, sem):
        return pltpu.make_async_copy(src.at[:, _ds(j * 128, 128)], dst.at[j].bitcast(BF), sem)

    def x_copy(r0, n, sem):
        return [pltpu.make_async_copy(x_hbm.at[pl.ds(r0, n), pl.ds(j * 128, 128)],
                                      xin.at[j, pl.ds(r0 // 2, n // 2)].bitcast(BF), sem) for j in range(G)]

    def out_copies(r0, n):
        return [pltpu.make_async_copy(xout.at[g, _ds(r0 // 2, n // 2)].bitcast(BF),
                                      out_hbm.at[_ds(r0, n), pl.ds(g * 128, 128)], osem) for g in range(G)]

    def flush(cond, b, n=1):
        @pl.when(cond)
        def _():
            for c in out_copies(b * R, n * R):
                c.start()

    cp_x = [x_copy(0, R, xsem.at[0]),
            x_copy(R, 2 * R, xsem.at[1]) + [pltpu.make_async_copy(wr_hbm, wr_in, xsem.at[1])],
            x_copy(3 * R, 2 * R, xsem.at[2]),
            x_copy(5 * R, S - 5 * R, xsem.at[3])]
    cp_w = [[col_copy(wqkv_hbm, wqkv, c * G + g, wsem.at[g]) for c in VKQ] for g in range(G)]
    cp_wo = [col_copy(wo_hbm, wo, j, wsem.at[G]) for j in range(G)]
    for c in cp_x[0] + cp_w[0] + cp_x[1]:
        c.start()

    for g in range(G):
        qkv_s[g][ROWS + 32:ROWS + 40, _L(0)] = jnp.zeros((8, 128), U32)

    def clear(i, c):
        xs[:, _ds(i * R, R), :] = jnp.zeros((G, R, 128), F32)
        return c
    lax.fori_loop(0, NB, clear, 0)

    tri = lax.broadcasted_iota(jnp.int32, (32, 128), 0) > (lax.broadcasted_iota(jnp.int32, (32, 128), 1) & 31)
    lane = lax.broadcasted_iota(jnp.int32, (16, 128), 1)
    row = lax.broadcasted_iota(jnp.int32, (16, 128), 0)
    u0 = jnp.zeros((16, 128), U32)
    tri_p = (jnp.where(2 * row > (lane & 31), np.uint32(0x0000FFFF), u0)
             | jnp.where(2 * row + 1 > (lane & 31), np.uint32(0xFFFF0000), u0))
    head_of_lane = lane // DH
    odd = (lane & 32) != 0
    upper = (lane & 64) != 0

    def rotate4(ts, zero):
        n = zero.shape[0]

        def sel(m, a, b):
            if a is None and b is None:
                return None
            return jnp.where(m[0:n], zero if a is None else a, zero if b is None else b)
        a = [sel(odd, ts[(1 - k) % 4], ts[-k % 4]) for k in range(4)]
        return [sel(upper, a[(h - 2) % 4], a[h]) for h in range(4)]

    def resid(first, g, r0):
        x = _up(xin[g, _ds(r0 // 2, 8), :]).astype(F32)
        return jnp.where(first, x, xs[g, _ds(r0, 16), :])

    def wide(col):
        return jnp.broadcast_to(col[0:8] + col[8:16], (8, 128))

    def ln_items(load, dst, d0):
        m = _rowsum([load(g) for g in range(G)]) * (1.0 / D)
        yield wide(m)
        xc = [load(g) - m for g in range(G)]
        ss = _rowsum([c * c for c in xc])
        yield wide(ss)
        rs = lax.rsqrt(ss * (1.0 / D) + EPS)
        yield wide(rs)
        for g in range(G):
            y = (load(g) - m) * rs
            dst.bitcast(BF)[d0:d0 + EP, _L(g)] = y.astype(BF)
            if g % 4 == 3:
                yield y[8:16]

    def epi_items(b, j, src):
        r0 = b * R + j * EP
        load = lambda g: src[g, j * EP:(j + 1) * EP, :]
        m = _rowsum([load(g) for g in range(G)]) * (1.0 / D)
        yield wide(m)
        xc = [load(g) - m for g in range(G)]
        ss = _rowsum([c * c for c in xc])
        yield wide(ss)
        r = _rowsum([(load(g) - m) * wr_s[g] for g in range(G)])
        yield wide(r)
        rs = lax.rsqrt(ss * (1.0 / D) + EPS)
        r = r * rs
        take = r > st_f[0]
        st_f[0] = jnp.where(take, r, st_f[0])
        st_f[1] = jnp.where(take, rs, st_f[1])
        st_i[...] = jnp.where(take, lax.broadcasted_iota(jnp.int32, (EP, 1), 0) + r0, st_i[...])
        yield wide(r)
        for g in range(G):
            x = load(g)
            x2 = x + (x - m) * rs
            xs[g, _ds(r0, EP), :] = x2
            packed = pltpu.bitcast(x2.astype(BF), U32)
            xout[g, _ds(r0 // 2, EP // 2), :] = packed
            if g % 2 == 1:
                yield pltpu.bitcast(packed, F32)

    chunks = [slice(i * 16, (i + 1) * 16) for i in range(R // 16)]

    def halves(src, w, j):
        return [jnp.dot(_up(src[:, h * D // 2:(h + 1) * D // 2]), _up(w[j, h * D // 4:(h + 1) * D // 4, :]),
                        preferred_element_type=F32) for h in range(2)]

    def qkv_pieces(zero, src, b, g, between=None):
        def mark(y):
            if zero is not None:
                qkv_s[g][_ds(ROWS + 8 + zero, 8), _L(0)] = pltpu.bitcast(y[8:16], U32)

        def put(col, i, y):
            qkv_b[g][_ds((W if col else 0) + b * R + i * 16, 16), _L(col)] = y.astype(BF)
        vt = []

        def piece(col):
            y0, y1 = halves(src, wqkv, col * G + g)
            if col == 2 and between is not None:
                between()
            for r in chunks:
                mark(y0[r])
                yield
            y = y0 + y1
            if col == 2:
                vt.append(y.astype(BF).T)
            for i, r in enumerate(chunks):
                if col == 2:
                    mark(y[r])
                else:
                    put(col, i, y[r] * QSCALE if col == 0 else y[r])
                if col == 1 and i == len(chunks) - 1:
                    for k, rk in enumerate(chunks):
                        put(2, k, vt[0][rk])
                yield
        return [piece(col) for col in VKQ]

    def o_piece(first, b, g, src, dst, ln_block=None):
        y0, y1 = halves(src, wo, g)
        for i, r in enumerate(chunks):
            dst[g, r, :] = resid(first, g, b * R + i * 16) + y0[r]
            yield
        for i, r in enumerate(chunks):
            dst[g, r, :] = dst[g, r, :] + y1[r]
            if ln_block is not None:
                ln_s[g, r, :] = resid(first, g, ln_block * R + i * 16)
            yield

    def qk_piece(b, g):
        res = []
        for c in range(4):
            q = qkv_s[g][_ds(b * 64 + c * 16, 16), _L(0)]
            w = _up(jnp.concatenate([jnp.where(head_of_lane == (l - c) % 4, q, u0) for l in range(4)], axis=0))
            skip = max(0, 8 - 4 * b - c) if isinstance(b, int) else 0
            k0 = b * 64 + 16 * (c + skip)
            k0 = k0 if isinstance(k0, int) else pl.multiple_of(k0, 16)
            kk = _up(qkv_s[g][pl.ds(k0, 16 * (9 - skip)), _L(1)])
            sc = lax.dot_general(kk, w, NT, preferred_element_type=F32)
            e = jnp.where(tri, NEG if skip else sc[0:32], sc[-32:])
            mid = sc[(0 if skip else 32):-32]
            t = jnp.concatenate([mid, e], axis=0) if mid.shape[0] else e
            res.append((t, jnp.max(t, axis=0, keepdims=True)))
        return res

    def exp_work(g, sc, get_max, sums, off):
        for i, (t, _) in enumerate(sc):
            acc = None
            for u in range(t.shape[0] // 16):
                m = get_max(i)
                p = jnp.exp2(t[u * 16:(u + 1) * 16] - jnp.concatenate([m, m], axis=0))
                p_b[g][2 * off + u * 16:2 * off + (u + 1) * 16, _L(i)] = p.astype(BF)
                p = p[0:8] + p[8:16]
                acc = p if acc is None else acc + p
                yield
            sums.append(jnp.sum(acc, axis=0, keepdims=True))

    def softmax(li, g, sc, via, off=0):
        mx = [jnp.broadcast_to(m, (8, 128)) for _, m in sc]
        sums = []
        if isinstance(via, int):
            idx = lambda i: (_ds(ROWS + 40 + 32 * li + 8 * i, 8), _L(1 if off else 0))
            for i in range(4):
                qkv_s[via][idx(i)] = pltpu.bitcast(mx[i], U32)
            get_max = lambda i: pltpu.bitcast(qkv_s[via][idx(i)], F32)
        else:
            idx = lambda i: (G - 1, _ds(R + 32 * li + 8 * i, 8), slice(None))
            for i in range(4):
                via[idx(i)] = mx[i]
            get_max = lambda i: via[idx(i)]
        return (sum(x.shape[0] // 16 for x, _ in sc), exp_work(g, sc, get_max, sums, off)), sums

    def pv_piece(b, g, sc, sums, dst, d0, off=0):
        def chunk(c, j):
            n = sc[c][0].shape[0] // 32
            if j < 0 or j > 8 or (n < 8 and j < 9 - n):
                return None
            if j in (0, 8):
                pe = p_s[g][pl.ds(off + 16 * (n - 1), 16), _L(c)]
                return pe & tri_p if j == 0 else pe & ~tri_p
            return p_s[g][pl.ds(off + 16 * (j - 9 + n), 16), _L(c)]
        outs = [None] * 4
        for kt in range(max(0, 2 - b) if isinstance(b, int) else 0, 3):
            ps = [rotate4([chunk(c, pos - c) for c in range(4)], u0) for pos in range(4 * kt, 4 * kt + 4)]
            for h in range(4):
                p = _up(jnp.concatenate([x[h] for x in ps], axis=0))
                vt = _up(qkv_s[g][_ds((b + kt) * 64 + h * 16, 16), _L(2)])
                o = jnp.dot(vt, p, preferred_element_type=F32)
                outs[h] = o if outs[h] is None else outs[h] + o
        inv = rotate4([1.0 / s for s in sums], sums[0])
        outs = [outs[h] * inv[h] for h in range(4)]
        outs = [o if h == 0 else pltpu.roll(o, 128 - 32 * h, axis=1) for h, o in enumerate(outs)]
        dst.bitcast(BF)[_ds(d0, R), _L(g)] = jnp.concatenate(outs, axis=0).astype(BF).T

    def paced(pieces, works, after=None):
        nwork = sum(n for n, _ in works)
        work = (None for _, w in works for _ in w)
        nch, done, ch = len(pieces) * CH, 0, 0
        for pc in pieces:
            for _ in pc:
                ch += 1
                while done < nwork * ch // nch:
                    next(work)
                    done += 1
                if after is not None:
                    after()
        _drain(work)

    def prologue(li):
        first = li == 0
        zero = 8 * (li // 2)

        def sync(wait, start):
            @pl.when(first)
            def _():
                for c in wait[:-1]:
                    c.wait()
                for c in start:
                    c.start()
                wait[-1].wait()

        def ln_block(b, dst, d0, js=range(R // EP)):
            for j in js:
                x = [resid(first, g, b * R + j * EP) for g in range(G)]
                _drain(ln_items(lambda g: x[g], dst, d0 + j * EP))

        plan = {0: (cp_w[0] + cp_x[1], cp_w[2]),
                1: (cp_w[1] + cp_w[2], cp_w[3] + cp_w[4] + cp_w[5]),
                3: (cp_w[3] + cp_w[4], cp_w[6] + cp_w[7] + cp_x[2]),
                5: (cp_w[5] + cp_w[6] + cp_w[7] + cp_x[2], cp_wo)}
        sync(cp_x[0], cp_w[1])
        ln_block(0, xn0, 0)
        sc = None
        for g in range(G + 1):
            if g in plan:
                sync(*plan[g])
            if g == 0:
                ln_block(1, xn0, R)
                ln_block(2, xn0, 2 * R)
            if g == 1:
                for i in range(G):
                    wr_s[i] = jnp.broadcast_to(wr_in[i:i + 1, :].astype(F32), (EP, 128))
            pieces = []
            for b in range(3 if g < G else 0):
                marked = (0 < g and b < 2) or g == G - 1
                pieces += qkv_pieces(zero if marked else None, xn0.at[pl.ds(b * R // 2, R // 2)], b, g)
            sm = [softmax(li, g - 1, sc[b], min(g, G - 1), 128 * b) for b in range(2)] if g else []
            if g == G - 1:
                late, pieces = pieces[6:], pieces[:6]
            paced(pieces[:5] if g < G else late[:1], [w for w, _ in sm])
            for pc in pieces[5:7] if g < G else late[1:2]:
                _drain(pc)
            cur, sc = sc, [qk_piece(b, g) for b in range(2)] if g < G else None
            for b, (_, sums) in enumerate(sm):
                pv_piece(b, g - 1, cur[b], sums, o_s, b * R, 128 * b)
            for pc in pieces[7:] if g < G else late[2:]:
                _drain(pc)
            if g in (5, 6):
                ln_block(3, xn_new, 0, range(4 * (g - 5), 4 * (g - 4)))

    def step(li, t):
        first = li == 0
        ln_block = jnp.minimum(t + 2, NB - 1)
        slot = t % 2
        o_prev = o_s.at[_ds(slot * (R // 2), R // 2)]
        zero = 8 * (li // 2)

        def o_and_copy(i):
            xn_cur[:, _L(i)] = xn_new[:, _L(i)]
            x1_s[1, _ds(R + 32 * li, 8), :] = pltpu.bitcast(xn_cur[_ds(zero, 8), _L(i)], F32)
            if i == 1:
                @pl.when(first & (t == 2))
                def _():
                    for cp in cp_x[3]:
                        cp.start()
            if i == 2:
                flush((li == 1) & (t >= 3), jnp.maximum(t - 3, 0))
            if i == 3:
                @pl.when(first & (t >= 3) & (t < 3 + FT // 4))
                def _():
                    for j in range(4):
                        col_copy(wg_hbm, wg, (t - 3) * 4 + j, fsem).start()
                        col_copy(wu_hbm, wu, (t - 3) * 4 + j, fsem).start()

                @pl.when(first & (t >= 3) & (t < 3 + G))
                def _():
                    col_copy(wd_hbm, wd, t - 3, fsem).start()
            yield from o_piece(first, t - 2, i, o_prev, x1_s, ln_block)

        def in_pairs(gens):
            for a, b in zip(gens[0::2], gens[1::2]):
                for x in a:
                    yield x
                    yield next(b)

        n_items = N_LN + N_EPI
        epi = in_pairs([epi_items(t - 2, j, x1_s) for j in range(R // EP)])
        ln = in_pairs([ln_items(lambda g, j=j: ln_s[g, j * EP:(j + 1) * EP, :], xn_new, j * EP)
                       for j in range(R // EP)])
        items = [(ln_s, ln) if k * N_LN // n_items != (k + 1) * N_LN // n_items else (x1_s, epi)
                 for k in range(n_items)]
        pending = []
        point = [0]

        def after(q):
            point[0] += 1
            while pending and pending[0][0] <= point[0]:
                q[_ds(ROWS + zero, 8), _L(0)] = pltpu.bitcast(pending.pop(0)[1], U32)
            if items and n_items - len(items) < n_items * point[0] // SPREAD:
                ref, gen = items.pop(0)
                ref[0, _ds(R + 32 * li, 8), :] = pltpu.bitcast(q[ROWS + 32:ROWS + 40, _L(0)], F32)
                pending.append((point[0] + LAG, next(gen)))

        _drain(o_and_copy(0))
        sc = qk_piece(t, 0)
        for g in range(G):
            if g == 0:
                pieces = [o_and_copy(i) for i in range(1, G)]
            else:
                pieces = qkv_pieces(zero, xn_cur, t + 1, g - 1)
            work, sums = softmax(li, g, sc, g - 1 if g else x1_s)
            paced(pieces, [work], (lambda: after(qkv_s[g - 1])) if g else None)
            cur = sc
            if g + 1 < G:
                sc = qk_piece(t, g + 1)
                pv_piece(t, g, cur, sums, o_s, slot * R)
        paced(qkv_pieces(zero, xn_cur, t + 1, G - 1, lambda: pv_piece(t, G - 1, cur, sums, o_s, slot * R)),
              [], lambda: after(qkv_s[G - 1]))
        assert not items

    def tail(li):
        first = li == 0
        t = NB - 1
        fill = ([o_piece(first, t - 2, g, o_s.at[pl.ds(R // 2, R // 2)], x1_s) for g in range(G)]
                + [o_piece(first, t - 1, g, o_s.at[pl.ds(0, R // 2)], ln_s) for g in range(G)])
        cuts = (0, 2, 4, 6, 8, 10, 12, 13, 14)

        def pace(ref, tok):
            ref[0, _ds(R + 32 * li, 8), :] = tok

        sc = qk_piece(t, 0)
        for g in range(G):
            work, sums = softmax(li, g, sc, x1_s if g < 4 else ln_s)
            paced(fill[cuts[g]:cuts[g + 1]], [work])
            cur = sc
            if g + 1 < G:
                sc = qk_piece(t, g + 1)
            else:
                _drain(fill[14])
            pv_piece(t, g, cur, sums, xn_cur, 0)
            if 3 <= g < 7:
                pace(x1_s, jnp.broadcast_to(sums[0], (8, 128)))
                _drain(epi_items(t - 2, 2 * g - 6, x1_s))
                _drain(epi_items(t - 2, 2 * g - 5, x1_s))
        _drain(fill[15])
        for g in range(G):
            _drain(epi_items(t - 1, g, ln_s))
            _drain(o_piece(first, t, g, xn_cur, x1_s))
            pace(ln_s, x1_s[g, R - 8:R, :])
        for j in range(R // EP):
            _drain(epi_items(t, j, x1_s))

    def routed_ffn():
        best = st_f[0]
        rmax = jnp.max(best, axis=0, keepdims=True)
        cand = jnp.where(best == rmax, st_i[...], S - 1)
        imin = jnp.min(cand, axis=0, keepdims=True)
        rs = jnp.max(jnp.where(cand == imin, st_f[1], 0.0), axis=0, keepdims=True)
        idx = jnp.clip(jnp.min(cand), 0, S - 1)
        t0 = (idx // 16) * 16

        x2 = [xs[g, pl.ds(idx, 1), :] for g in range(G)]
        m = _rowsum(x2) * (1.0 / D)
        xrow = [((x - m) * (rs / (1.0 + rs))).astype(BF).astype(F32) for x in x2]
        xsel = jnp.concatenate([jnp.broadcast_to(x, (16, 128)) for x in xrow], axis=1).astype(BF)
        for g in range(G):
            ln_s[g, 0:128, :] = jnp.broadcast_to(xrow[g], (128, 128)).T

        def vpu_matvec(tiles):
            acc = [None] * len(tiles)
            for k in range(D // 16):
                x_even = ln_s[k // 8, pl.ds((k % 8) * 16, 8, stride=2), :]
                x_odd = ln_s[k // 8, pl.ds((k % 8) * 16 + 1, 8, stride=2), :]
                for i, (w, j) in enumerate(tiles):
                    u = w[j, k * 8:(k + 1) * 8, :]
                    p = (pltpu.bitcast(u << 16, F32) * x_even
                         + pltpu.bitcast(u & np.uint32(0xFFFF0000), F32) * x_odd)
                    acc[i] = p if acc[i] is None else acc[i] + p
            return [jnp.sum(a, axis=0, keepdims=True) for a in acc]

        y = [None] * G

        def down(j, gt, ut):
            h = jnp.broadcast_to(gt * jax.nn.sigmoid(gt) * ut, (16, 128)).astype(BF)
            for g in range(G):
                p = jnp.dot(h, _up(wd[g, j * 64:(j + 1) * 64, :]), preferred_element_type=F32)[0:8]
                y[g] = p if y[g] is None else y[g] + p

        ready = []
        for j0 in range(0, FT, 7):
            for j in range(j0, j0 + 7 - NV):
                ready.append((j, jnp.dot(xsel, _up(wg[j]), preferred_element_type=F32)[0:1],
                              jnp.dot(xsel, _up(wu[j]), preferred_element_type=F32)[0:1]))
            while ready:
                down(*ready.pop(0))
            for j in range(j0 + 7 - NV, j0 + 7, 2):
                r = vpu_matvec([(w, jj) for jj in (j, j + 1) for w in (wg, wu)])
                ready += [(j, r[0], r[1]), (j + 1, r[2], r[3])]
        while ready:
            down(*ready.pop(0))
        gate = jax.nn.sigmoid(rmax)
        sel = lax.broadcasted_iota(jnp.int32, (16, 128), 0) == (idx - t0)
        return t0, [xs[g, _ds(t0, 16), :] + jnp.where(sel, y[g][0:1] * gate, 0.0) for g in range(G)]

    def layer(li, carry):
        st_f[0] = jnp.full((EP, 1), -jnp.inf, F32)
        st_f[1] = jnp.zeros((EP, 1), F32)
        st_i[...] = jnp.zeros((EP, 1), jnp.int32)
        prologue(li)

        def steady(t, c):
            for when, cps in ((2, cp_wo), (3, cp_x[3])):
                @pl.when((li == 0) & (t == when))
                def _():
                    for cp in cps:
                        cp.wait()
            step(li, t)
            return c
        lax.fori_loop(2, NB - 1, steady, 0)

        @pl.when(li == 0)
        def _():
            def gate_up(j, c):
                col_copy(wg_hbm, wg, j, fsem).wait()
                col_copy(wu_hbm, wu, j, fsem).wait()
                return c

            def down(j, c):
                col_copy(wd_hbm, wd, j, fsem).wait()
                return c
            lax.fori_loop(0, FT, gate_up, 0)
            lax.fori_loop(0, G, down, 0)

        flush(li == 1, NB - 4)
        tail(li)
        flush(li == 1, NB - 3, 3)

        t0, x3 = routed_ffn()
        for g in range(G):
            xs[g, _ds(t0, 16), :] = x3[g]

        @pl.when(li == 1)
        def _():
            def wait_block(b, c):
                for cp in out_copies(b * R, R):
                    cp.wait()
                return c
            lax.fori_loop(0, NB - 3, wait_block, 0)
            for cp in out_copies((NB - 3) * R, 3 * R):
                cp.wait()
            for g in range(G):
                xout[g, _ds(t0 // 2, 8), :] = pltpu.bitcast(x3[g].astype(BF), U32)
            cps = out_copies(t0, 16)
            for cp in cps:
                cp.start()
            for cp in cps:
                cp.wait()
        return carry

    lax.fori_loop(0, 2, layer, 0)


@jax.jit
def pallas_interleave_layers__sliding_block__moe_arch_mod__prompt_kernel(
    A_x: jax.Array,
    A_wqkv: jax.Array,
    A_wo: jax.Array,
    B_x: jax.Array,
    B_w_r: jax.Array,
    B_w_gate: jax.Array,
    B_w_up: jax.Array,
    B_w_down: jax.Array,
):
    del B_x
    any_spec = pl.BlockSpec(memory_space=pl.ANY)
    out = pl.pallas_call(
        _kernel,
        out_shape=jax.ShapeDtypeStruct((S, D), BF),
        in_specs=[any_spec] * 7,
        out_specs=any_spec,
        scratch_shapes=[
            pltpu.VMEM((G, S // 2, 128), U32),
            pltpu.VMEM((G, S // 2, 128), U32),
            pltpu.VMEM((G, S, 128), F32),
            pltpu.VMEM((3 * R // 2, D), U32),
            pltpu.VMEM((R // 2, D), U32),
            pltpu.VMEM((R // 2, D), U32),
            pltpu.VMEM((3 * G, D // 2, 128), U32),
            pltpu.VMEM((G, D // 2, 128), U32),
            pltpu.VMEM((FT, D // 2, 128), U32),
            pltpu.VMEM((FT, D // 2, 128), U32),
            pltpu.VMEM((G, F // 2, 128), U32),
            pltpu.VMEM((R, D), U32),
            pltpu.VMEM((G, R + 64, 128), F32),
            pltpu.VMEM((G, R + 64, 128), F32),
            pltpu.VMEM((G, 128), BF),
            pltpu.VMEM((G, EP, 128), F32),
            pltpu.VMEM((2, EP, 1), F32),
            pltpu.VMEM((EP, 1), jnp.int32),
            pltpu.SemaphoreType.DMA((4,)),
            pltpu.SemaphoreType.DMA((G + 1,)),
            pltpu.SemaphoreType.DMA(()),
            pltpu.SemaphoreType.DMA(()),
        ] + [pltpu.VMEM((ROWS + 104, 384), U32)] * G
          + [pltpu.VMEM((256, 512), U32)] * G,
        compiler_params=pltpu.CompilerParams(vmem_limit_bytes=120 * 2**20, disable_bounds_checks=True),
        name="kern",
    )(A_x.reshape(S, D), A_wqkv, A_wo, B_w_r.reshape(G, 128), B_w_gate, B_w_up, B_w_down)
    return out.reshape(1, S, D)
```
